```python
import os as _os
_os.environ.setdefault('JAX_PLATFORMS', 'cpu')
import jax
import jax.numpy as jnp

def _softmax(x, axis=-1):
    return jax.nn.softmax(x, axis=axis)

def _gelu(x):
    return jax.nn.gelu(x, approximate=True)

def _silu(x):
    return jax.nn.silu(x)

def _sigmoid(x):
    return jax.nn.sigmoid(x)

def _layernorm(x, axis=-1, eps=1e-05):
    m = jnp.mean(x, axis=axis, keepdims=True)
    v = jnp.var(x, axis=axis, keepdims=True)
    return (x - m) / jnp.sqrt(v + eps)

def _scatter_add(tgt, idx, src, axis=0):
    return tgt.at[idx].add(src)

def _segment_sum(src, seg, n):
    return jax.ops.segment_sum(src, seg, n)

class _Rng:

    def __init__(self, key):
        self._k = key

    def _next(self):
        self._k, sub = jax.random.split(self._k)
        return sub

    def normal(self, shape):
        return jax.random.normal(self._next(), shape, dtype=jnp.bfloat16)

    def randint(self, lo, hi, shape):
        return jax.random.randint(self._next(), shape, lo, hi, dtype=jnp.int32)

    def uniform(self, shape, lo=0.0, hi=1.0):
        return jax.random.uniform(self._next(), shape, jnp.bfloat16, lo, hi)

    def permutation(self, n):
        return jax.random.permutation(self._next(), n)
kernel_name = 'standalone__conformer_conv_module__speech'

def setup_inputs():
    _rng = _Rng(jax.random.key(int.from_bytes(__import__("os").urandom(4), "little")))
    _w = lambda a: (lambda t: t.astype(jnp.bfloat16) if jnp.issubdtype(t.dtype, jnp.floating) else t)(jnp.asarray(a))
    B, T, D, K = (2, 4000, 512, 15)
    return {'x': _w((lambda *s: _rng.normal(s) * 0.2)(B, T, D)), 'w_pw1': _w((lambda *s: _rng.normal(s) * 0.2)(D, 2 * D)), 'dw': _w((lambda *s: _rng.normal(s) * 0.05)(K, D)), 'w_pw2': _w((lambda *s: _rng.normal(s) * 0.05)(D, D))}

def reference(x, w_pw1, dw, w_pw2):
    B, T, D = x.shape
    K = dw.shape[0]
    h = x @ w_pw1
    a, b = (h[..., :D].copy(), h[..., D:].copy())
    h = a * _sigmoid(b)
    pad = K // 2
    hp = jnp.pad(h, ((0, 0), (pad, pad), (0, 0)))
    out = jnp.zeros_like(h)
    for i in range(K):
        out = out + hp[:, i:i + T, :] * dw[i][None, None, :]
    return _silu(out) @ w_pw2
```

```python
import functools
import jax
import jax.numpy as jnp
import jax.experimental.pallas as pl
import jax.experimental.pallas.tpu as pltpu

TM = 800
RC = 80

@jax.jit
def pallas_standalone__conformer_conv_module__speech_kernel(x, w_pw1, dw, w_pw2):
    B, T, D = x.shape
    K = dw.shape[0]
    pad = K // 2
    nt = T // TM
    N = B * nt
    NC = D // 128
    NQ = TM // RC
    f32 = jnp.float32
    bf16 = jnp.bfloat16
    u32 = jnp.uint32

    def kernel(x_ref, w1_ref, dw_ref, w2_ref, o_hbm, h_ref, dwb_ref, s_ref, w1p_ref, w2p_ref, obuf, sem):
        j = pl.program_id(0)
        sub = jax.lax.broadcasted_iota(jnp.int32, (8, 128), 0)

        @pl.when(j == 0)
        def _():
            dwf = dw_ref[...].astype(f32) * 0.25
            for c in range(NC):
                for k in range(K):
                    dwb_ref[c * K + k] = jnp.broadcast_to(dwf[k:k+1, c*128:(c+1)*128], (8, 128))
                h_ref[c, 0:16, :] = jnp.zeros((16, 128), f32)
            w1p_ref[...] = pltpu.bitcast(w1_ref[...], u32)
            w2p_ref[...] = pltpu.bitcast(w2_ref[...], u32)

        boundary = (j % nt) == 0

        def w1tile(col):
            return pltpu.bitcast(w1p_ref[:, col*128:(col+1)*128], bf16)
        def w2tile(col):
            return pltpu.bitcast(w2p_ref[:, col*128:(col+1)*128], bf16)

        def conv_vreg(c, ws, o, mode):
            acc = None
            for k in range(K):
                v = h_ref[c, pl.ds(16 + o + k - pad, 8), :]
                if mode == 'prev' and k >= 8:
                    thr = jnp.where(boundary, 15 - k, 8)
                    v = jnp.where(sub < thr, v, 0.0)
                elif mode == 'prev_static' and k >= 8:
                    v = jnp.where(sub < 15 - k, v, 0.0)
                elif mode == 'next' and k <= 6:
                    thr = jnp.where(boundary, 7 - k, 0)
                    v = jnp.where(sub >= thr, v, 0.0)
                t = v * ws[k]
                acc = t if acc is None else acc + t
            return acc + acc * jnp.tanh(acc)

        obase = pl.multiple_of(j * TM, 16)
        ov = obuf.at[pl.ds(obase, TM), :]

        def mm2_pass(q, n):
            s = pltpu.bitcast(s_ref[q*RC//2:(q+1)*RC//2, :], bf16)
            return jnp.dot(s, w2tile(n), preferred_element_type=f32)

        def mm2_store(q, n, r0, r1):
            ov[q*RC:(q+1)*RC, (n-1)*128:(n+1)*128] = jnp.concatenate([r0, r1], axis=1).astype(bf16)

        def out_dma(q):
            if q > 0:
                src = pl.multiple_of(j * TM + (q - 1) * RC + 8, 8)
                dst = pl.multiple_of(j * TM + (q - 1) * RC, 8)
                pltpu.make_async_copy(obuf.at[pl.ds(src, RC), :], o_hbm.at[pl.ds(dst, RC), :], sem).start()
            else:
                pass

        for q in range(NQ):
            xq = x_ref[q*RC:(q+1)*RC, :]
            rprev = None
            for c in range(NC):
                a = jnp.dot(xq, w1tile(c), preferred_element_type=f32)
                b = jnp.dot(xq, w1tile(NC + c), preferred_element_type=f32)
                g = a * (1.0 + jnp.tanh(0.5 * b))
                h_ref[c, 16 + q*RC:16 + (q+1)*RC, :] = g
                ws = [dwb_ref[c * K + k] for k in range(K)]
                for p in range(RC // 16):
                    o = q * RC - 8 + 16 * p
                    m0 = 'prev' if (q == 0 and p == 0) else None
                    m1 = 'next' if (q == 0 and p == 0) else None
                    s0 = conv_vreg(c, ws, o, m0)
                    s1 = conv_vreg(c, ws, o + 8, m1)
                    sp = jnp.concatenate([s0, s1], axis=0).astype(bf16)
                    s_ref[(q*RC + 16*p)//2:(q*RC + 16*p)//2 + 8, c*128:(c+1)*128] = pltpu.bitcast(sp, u32)
                if q > 0:
                    r = mm2_pass(q - 1, c)
                    if c % 2 == 1:
                        mm2_store(q - 1, c, rprev, r)
                    rprev = r
            if q > 0:
                out_dma(q - 1)
        for c in range(NC):
            r = mm2_pass(NQ - 1, c)
            if c % 2 == 1:
                mm2_store(NQ - 1, c, rprev, r)
            rprev = r
        out_dma(NQ - 1)
        for c in range(NC):
            h_ref[c, 0:16, :] = h_ref[c, TM:TM + 16, :]

        @pl.when(j > 0)
        def _():
            src = pl.multiple_of(j * TM - RC + 8, 8)
            dst = pl.multiple_of(j * TM - RC, 8)
            pltpu.make_async_copy(obuf.at[pl.ds(src, RC), :], o_hbm.at[pl.ds(dst, RC), :], sem).start()

        @pl.when(j == N - 1)
        def _():
            parts = []
            for c in range(NC):
                ws = [dwb_ref[c * K + k] for k in range(K)]
                parts.append(conv_vreg(c, ws, -8, 'prev_static'))
            s = jnp.concatenate(parts, axis=1).astype(bf16)
            w2 = pltpu.bitcast(w2p_ref[...], bf16)
            obuf[N*TM:N*TM + 8, :] = jnp.dot(s, w2, preferred_element_type=f32).astype(bf16)
            pltpu.make_async_copy(obuf.at[pl.ds(N * TM - RC + 8, RC), :], o_hbm.at[pl.ds(N * TM - RC, RC), :], sem).start()
            pltpu.make_async_copy(o_hbm, o_hbm, sem).wait()

    x2 = x.reshape(B * T, D)
    out = pl.pallas_call(
        kernel,
        grid=(N,),
        in_specs=[
            pl.BlockSpec((TM, D), lambda j: (j, 0)),
            pl.BlockSpec((D, 2 * D), lambda j: (0, 0)),
            pl.BlockSpec((K, D), lambda j: (0, 0)),
            pl.BlockSpec((D, D), lambda j: (0, 0)),
        ],
        out_specs=pl.BlockSpec(memory_space=pl.ANY),
        out_shape=jax.ShapeDtypeStruct((B * T, D), x.dtype),
        scratch_shapes=[
            pltpu.VMEM((NC, 16 + TM, 128), f32),
            pltpu.VMEM((NC * K, 8, 128), f32),
            pltpu.VMEM((TM // 2, D), u32),
            pltpu.VMEM((D // 2, 2 * D), u32),
            pltpu.VMEM((D // 2, D), u32),
            pltpu.VMEM((B * T + 16, D), bf16),
            pltpu.SemaphoreType.DMA,
        ],
        compiler_params=pltpu.CompilerParams(
            dimension_semantics=("arbitrary",),
            vmem_limit_bytes=100 * 1024 * 1024),
    )(x2, w_pw1, dw, w_pw2)
    return out.reshape(B, T, D)
```

```python
import jax
import jax.numpy as jnp
import jax.experimental.pallas as pl
import jax.experimental.pallas.tpu as pltpu

RC = 80
QP = 12
NP = 6
XA = 176
QB = 44
MLAG = 6
DEADLINE = 3
SDL = 2
SLAG = 1
RESV = 21
XDEP = 1
BORD = (0, 1, 2, 3, 1, 0, 3, 2)
IORD = (0, 2, 4, 1, 3)
KDEP = 14
LAGSC = 2
XU = 5
XU0 = 7
XH = 12
XDL = 2
T1 = (0, 2)
T2 = (1, 3)


@jax.jit
def pallas_standalone__conformer_conv_module__speech_kernel(x, w_pw1, dw, w_pw2):
    B, T, D = x.shape
    K = dw.shape[0]
    pad = K // 2
    R = B * T
    NC = D // 128
    TP = QP * RC
    TB = QB * RC
    NB = (R - TP) // TB
    assert TP + NB * TB == R and T % RC == 0 and B == 2 and TP < T and pad <= 8 and NC == 4
    gq = (T - TP) // RC
    bnd_it, bnd_q = gq // QB, gq % QB
    f32, bf16, u32 = jnp.float32, jnp.bfloat16, jnp.uint32
    HR = max(TP, TB) + 16
    NPAIR = RC // 16
    X0 = NP * RC + 16
    X1 = TP + 8 * NB
    XN = TB - 8

    def kernel(x_hbm, w1_hbm, dw_hbm, w2_hbm, o_hbm,
               xbuf, w1raw, w2raw, dwraw, w1p, w2p, dwb, h_ref, s_all, obuf,
               wsa, wsm, xs_all, xr_all, ss_all, g_all, sem_in, sem_x, sem_out):
        j = pl.program_id(0)
        sub = jax.lax.broadcasted_iota(jnp.int32, (16, 128), 0)
        never = sub > j + 1000
        s_ref = s_all.at[j % 2]
        xs_ref, xr_ref, ss_ref, g_ref = xs_all.at[j % 2], xr_all.at[j % 2], ss_all.at[j % 2], g_all.at[j % 2]
        RH = RC // 2

        def st_packed(ref, r, t, v):
            ref[r:r + 8, t * 128:(t + 1) * 128] = pltpu.bitcast(v.astype(bf16), u32)

        def w1_copy(col, s):
            return pltpu.make_async_copy(w1_hbm.at[:, pl.ds(col * 128, 128)], w1raw.at[col], sem_in.at[s])

        def w2_copy(col, s):
            return pltpu.make_async_copy(w2_hbm.at[:, pl.ds(col * 128, 128)], w2raw.at[col], sem_in.at[s])

        def x_copy(lo, hi, s):
            return pltpu.make_async_copy(x_hbm.at[pl.ds(lo, hi - lo), :], xbuf.at[pl.ds(lo, hi - lo), :], sem_in.at[s])

        groups = [
            [x_copy(0, XA, 0), w1_copy(0, 0), w1_copy(NC, 0)],
            [x_copy(XA, X0, 1), pltpu.make_async_copy(dw_hbm, dwraw, sem_in.at[1])],
            [w1_copy(1, 2), w1_copy(NC + 1, 2)],
            [w1_copy(2, 3), w1_copy(NC + 2, 3), w1_copy(3, 3), w1_copy(NC + 3, 3)],
            [w2_copy(n, 4) for n in range(NC)] + [x_copy(X0, X1, 4)],
        ]

        def wait_group(g):
            for cp in groups[g]:
                cp.wait()

        def xb_copy(i):
            lo = X1 + i * XN
            if not isinstance(lo, int):
                lo = pl.multiple_of(lo, 8)
            return pltpu.make_async_copy(x_hbm.at[pl.ds(lo, XN), :], xbuf.at[pl.ds(lo, XN), :], sem_x)

        def w1tile(col, raw=False):
            if raw:
                wt = w1raw[col]
                w1p[:, col * 128:(col + 1) * 128] = pltpu.bitcast(wt, u32)
                return wt
            return pltpu.bitcast(w1p[:, col * 128:(col + 1) * 128], bf16)

        def w2tile(col, raw=False):
            if raw:
                wt = w2raw[col]
                w2p[:, col * 128:(col + 1) * 128] = pltpu.bitcast(wt, u32)
                return wt
            return pltpu.bitcast(w2p[:, col * 128:(col + 1) * 128], bf16)

        def conv16(c, o, mode, flag, dep, kdep, ws):
            acc = None
            for k in range(K):
                v = h_ref[c, pl.ds(8 + o + k - pad, 16), :]
                if mode == 'last' and k > pad:
                    v = jnp.where(sub < jnp.where(flag, 16 + pad - k, 16), v, 0.0)
                elif mode == 'first' and k < pad:
                    v = jnp.where(sub >= jnp.where(flag, pad - k, 0), v, 0.0)
                w = ws[k]
                if k == kdep and dep is not None:
                    w = jnp.where(never, dep, w)
                t = v * w
                acc = t if acc is None else acc + t
            return acc + acc * jnp.tanh(acc)

        class Blk:
            def __init__(self, xv, ov, obase, masks, kdep):
                self.xv, self.ov, self.obase, self.masks, self.kdep = xv, ov, obase, masks, kdep
                self.raw_w2 = False
                self.nq = 0
                self.xq, self.r, self.av, self.ws = {}, {}, {}, {}
                self.todo = []
                self.extra = []

            def conv_pair(self, q, c, p, dep):
                o = q * RC + 16 * p
                mode, flag = self.masks.get((q, p), (None, None))
                if (q, c) not in self.ws:
                    self.ws[(q, c)] = [jnp.concatenate([dwb[c * K + k]] * 2, axis=0) for k in range(K)]
                sp = conv16(c, o, mode, flag, dep, self.kdep, self.ws[(q, c)]).astype(bf16)
                s_ref[o // 2:o // 2 + 8, c * 128:(c + 1) * 128] = pltpu.bitcast(sp, u32)

            def attach(self, res, npairs):
                nv = res.shape[0] // 8
                npairs = min(npairs, len(self.todo))
                for i in range(npairs):
                    q, c, p = self.todo.pop(0)
                    i0 = (2 * i * nv) // (2 * npairs)
                    i1 = ((2 * i + 1) * nv) // (2 * npairs)
                    dep = jnp.concatenate([res[8 * i0:8 * i0 + 8], res[8 * i1:8 * i1 + 8]], axis=0)
                    self.conv_pair(q, c, p, dep)
                if self.extra and len(self.todo) <= 8:
                    wprep(*self.extra.pop(0), res[nv * 8 - 16:nv * 8])

            def run(self, kind, q, c, npairs):
                if kind == 'a':
                    if q not in self.xq:
                        self.xq[q] = self.xv[q * RC + 8:(q + 1) * RC + 8, :]
                    a = jnp.dot(self.xq[q], w1tile(c), preferred_element_type=f32)
                    self.av[(q, c)] = a
                    self.attach(a, npairs)
                elif kind == 'b':
                    b = jnp.dot(self.xq[q], w1tile(NC + c), preferred_element_type=f32)
                    self.attach(b, npairs)
                    h_ref[c, 16 + q * RC:16 + (q + 1) * RC, :] = self.av.pop((q, c)) * (1.0 + jnp.tanh(0.5 * b))
                    self.todo.extend((q, c, p) for p in range(NPAIR))
                else:
                    n = c
                    while any(it[0] <= q for it in self.todo):
                        self.conv_pair(*self.todo.pop(0), None)
                    s = pltpu.bitcast(s_ref[q * RC // 2:(q + 1) * RC // 2, :], bf16)
                    r = jnp.dot(s, w2tile(n, self.raw_w2 and q == 0), preferred_element_type=f32)
                    self.attach(r, npairs)
                    if n % 2 == 0:
                        self.r[q] = r
                    else:
                        self.ov[q * RC:(q + 1) * RC, (n - 1) * 128:(n + 1) * 128] = (
                            jnp.concatenate([self.r.pop(q), r], axis=1).astype(bf16))
                    if not isinstance(self.obase, int):
                        dst = pl.multiple_of(self.obase + q * RC, 16)
                        if q == self.nq - 1:
                            if n % 2 == 1:
                                cols = pl.ds((n - 1) * 128, 256)
                                pltpu.make_async_copy(self.ov.at[pl.ds(q * RC, RC), cols],
                                                      o_hbm.at[pl.ds(dst, RC), cols], sem_out).start()
                        elif n == NC - 1:
                            pltpu.make_async_copy(self.ov.at[pl.ds(q * RC, RC), :],
                                                  o_hbm.at[pl.ds(dst, RC), :], sem_out).start()

            def steady(self, q0, nq, pending):
                self.nq = nq
                seq = []
                ready = {q: MLAG - 1 for q in pending}
                pend = [(q, n) for q in pending for n in range(NC)]
                for q in range(q0, nq):
                    for c in range(NC):
                        seq.append(('a', q, c))
                        seq.append(('b', q, c))
                        if c == NC - 1:
                            ready[q] = len(seq) - 1 + MLAG
                            pend += [(q, n) for n in range(NC)]
                        k = 2 if len(pend) > 2 * NC + 2 else 1
                        if q == nq - 1:
                            k = 0 if len(pend) <= NC + (NC if c == NC - 1 else 0) else k
                        for _ in range(k):
                            if pend and ready[pend[0][0]] <= len(seq):
                                seq.append(('m',) + pend.pop(0))
                for it in pend:
                    seq.append(('m',) + it)
                first_m = {}
                for t, (kind, q, c) in enumerate(seq):
                    if kind == 'm' and q not in first_m:
                        first_m[q] = t
                for t, (kind, q, c) in enumerate(seq):
                    base = 1 if kind == 'b' else 2
                    n = base
                    if self.todo:
                        need = 0
                        for idx, it in enumerate(self.todo):
                            slots = max(first_m[it[0]] - DEADLINE - t + 1, 1)
                            need = max(need, -(-(idx + 1) // slots))
                        n = max(base, min(base + 2, need))
                        if len(self.todo) > 8:
                            n = max(n, base + 1)
                    self.run(kind, q, c, n)

            def carry(self, n):
                for c in range(NC):
                    h_ref[c, 0:16, :] = h_ref[c, n:n + 16, :]

        def wprep(which, l, kl, i, dep):
            if which == 'a':
                raw, dst, kt, nt = w1raw, wsa, ((0, 1), (2, 3)), (T1, T2)
            else:
                raw, dst, kt, nt = w2raw, wsm, (T1, T2), ((0, 2), (1, 3))

            def ld(kh, nh):
                r = kt[kh][kl] * 128 + 16 * i
                return raw[nt[nh][l], r:r + 16, :].astype(f32)
            b11, b12, b21, b22 = ld(0, 0), ld(0, 1), ld(1, 0), ld(1, 1)
            if dep is not None:
                b11 = jnp.where(never, dep, b11)
                b22 = jnp.where(never, dep, b22)
            for n, v in enumerate([b11 + b22, b11, b12 - b22, b21 - b11, b22, b11 + b12, b21 + b22]):
                st_packed(dst, n * 128 + kl * 64 + 8 * i, l, v)

        class SBlk:
            def __init__(self, xv, ov, obase, masks):
                self.xv, self.ov, self.obase, self.masks = xv, ov, obase, masks
                self.st = {}
                self.sv = {}

            def xprep(self, p, i, l, dep):
                def ld(q, t):
                    r = q * RC + 8 + 16 * i
                    cs = slice(t * 128, (t + 1) * 128)
                    return jnp.concatenate([self.xv[r:r + 8, cs].astype(f32),
                                            self.xv[r + 8:r + 16, cs].astype(f32)], axis=0)
                q1, q2 = 2 * p, 2 * p + 1
                a11, a12, a21, a22 = ld(q1, l), ld(q1, l + 2), ld(q2, l), ld(q2, l + 2)
                if dep is not None and XDEP:
                    a11 = jnp.where(never, dep, a11)
                    a22 = jnp.where(never, dep, a22)
                for n, v in enumerate([a11 + a22, a21 + a22, a11 + a12, a21 - a11, a12 - a22]):
                    st_packed(xs_ref, (p * 5 + n) * RH + 8 * i, l, v)
                for q, t, v in [(q1, l, a11), (q1, l + 2, a12), (q2, l, a21), (q2, l + 2, a22)]:
                    st_packed(xr_ref, q * RH + 8 * i, t, v)

            def cpair(self, p, l, i, half, dep):
                c = (T1, T2)[half][l]
                ws = [jnp.concatenate([dwb[c * K + k]] * 2, axis=0) for k in range(K)]
                out = []
                for u, q in enumerate((2 * p, 2 * p + 1)):
                    mode, flag = self.masks.get((q, i), (None, None))
                    out.append(conv16(c, q * RC + 16 * i, mode, flag, None if dep is None else dep[u], KDEP, ws))

                def put(n, v):
                    st_packed(ss_ref, (p * 7 + n) * RH + 8 * i, l, v)
                if half == 0:
                    s11, s21 = out
                    put(2, s11)
                    put(5, s21 - s11)
                    self.sv[(p, l, i)] = out
                else:
                    s11, s21 = self.sv.pop((p, l, i))
                    s12, s22 = out
                    put(0, s11 + s22)
                    put(1, s21 + s22)
                    put(3, s22)
                    put(4, s11 + s12)
                    put(6, s12 - s22)

            def lhs(self, kind, p, n):
                if kind == 'm':
                    v = ss_ref[(p * 7 + n) * RH:(p * 7 + n + 1) * RH, :]
                elif n == 2:
                    v = xr_ref[2 * p * RH:(2 * p + 1) * RH, 0:256]
                elif n == 3:
                    v = xr_ref[(2 * p + 1) * RH:(2 * p + 2) * RH, 256:512]
                else:
                    m = {0: 0, 1: 1, 4: 2, 5: 3, 6: 4}[n]
                    v = xs_ref[(p * 5 + m) * RH:(p * 5 + m + 1) * RH, :]
                return pltpu.bitcast(v, bf16)

            def prod(self, kind, p, n, l):
                w = (wsa if kind == 'a' else wsm)
                if l is None:
                    wt = w[n * 128:(n + 1) * 128, :]
                else:
                    wt = w[n * 128:(n + 1) * 128, l * 128:(l + 1) * 128]
                return jnp.dot(self.lhs(kind, p, n), pltpu.bitcast(wt, bf16), preferred_element_type=f32)

            def fin(self, kind, p, l, rh, ch, v):
                q = 2 * p + rh
                if kind == 'a':
                    c = (T1, T2)[ch][l]
                    g = g_ref[(q % 4) * RC:(q % 4 + 1) * RC, c * 128:(c + 1) * 128]
                    h_ref[c, 16 + q * RC:16 + (q + 1) * RC, :] = v * g
                else:
                    c = 2 * l + ch
                    self.ov[q * RC:(q + 1) * RC, c * 128:(c + 1) * 128] = v.astype(bf16)

            def run(self, kind, p, idx):
                if kind == 'b':
                    q, c = 2 * p + idx % 2, BORD[idx]
                    if p == 0:
                        xq = self.xv[q * RC + 8:(q + 1) * RC + 8, :]
                    else:
                        xq = pltpu.bitcast(xr_ref[q * RH:(q + 1) * RH, :], bf16)
                    b = jnp.dot(xq, w1tile(NC + c), preferred_element_type=f32)
                    g_ref[(q % 4) * RC:(q % 4 + 1) * RC, c * 128:(c + 1) * 128] = 1.0 + jnp.tanh(0.5 * b)
                    return b
                st = self.st.setdefault((kind, p), {})
                l = 0 if idx < 3 else 1
                step = idx if idx < 3 else idx - 4
                if idx == 3:
                    m6 = self.prod(kind, p, 5, None)
                    self.fin(kind, p, 0, 1, 1, st.pop('t22') + m6[:, 0:128])
                    st['t22'] = m6[:, 128:256]
                    return m6[:, 0:128]
                if step == 0:
                    m2, m4 = self.prod(kind, p, 1, l), self.prod(kind, p, 3, l)
                    self.fin(kind, p, l, 1, 0, m2 + m4)
                    st['t11'] = m4
                    st['t22'] = ('neg', m2) if l == 0 else st['t22'] - m2
                    return m2
                if step == 1:
                    m3, m5 = self.prod(kind, p, 2, l), self.prod(kind, p, 4, l)
                    self.fin(kind, p, l, 0, 1, m3 + m5)
                    st['t11'] = st['t11'] - m5
                    st['t22'] = m3 - st['t22'][1] if l == 0 else st['t22'] + m3
                    return m3
                m1, m7 = self.prod(kind, p, 0, l), self.prod(kind, p, 6, l)
                self.fin(kind, p, l, 0, 0, st.pop('t11') + m1 + m7)
                if l == 0:
                    st['t22'] = st['t22'] + m1
                else:
                    self.fin(kind, p, l, 1, 1, st.pop('t22') + m1)
                return m1

            def out_dma(self, p, cols):
                dst = pl.multiple_of(self.obase + 2 * p * RC, 16)
                pltpu.make_async_copy(self.ov.at[pl.ds(2 * p * RC, 2 * RC), cols],
                                      o_hbm.at[pl.ds(dst, 2 * RC), cols], sem_out).start()

            def steady(self, nsc):
                seq = []
                for p in range(nsc):
                    seq += [('b', p, i) for i in range(8)] + [('a', p, i) for i in range(7)]
                    if p >= LAGSC and 7 * (nsc - 1 - (p - LAGSC)) > RESV:
                        seq += [('m', p - LAGSC, i) for i in range(7)]
                done = {p for k, p, i in seq if k == 'm'}
                seq += [('m', p, i) for p in range(nsc) if p not in done for i in range(7)]
                pos = {it: t for t, it in enumerate(seq)}
                xs, cs = [], []
                for p in range(nsc):
                    dl = pos[('a', 0, 0)] - XDL if p == 0 else pos[('b', p, 0)] - XDL
                    xs += [(0, dl, (p, i, l)) for i in range(NPAIR) for l in range(2)]
                    dl = pos[('m', p, 0)] - SDL
                    for l in range(2):
                        for i in IORD:
                            for half in range(2):
                                av = pos[('a', p, (2 + half) if l == 0 else 6)] + SLAG
                                cs.append((av, dl, (p, l, i, half)))
                ncs, k = [], 0
                for t in range(len(seq)):
                    slack = min([it[1] - t - i for i, it in enumerate(cs[k:])], default=99)
                    n = len([it for it in cs[k:k + (2 if slack < 0 else 1)] if it[0] <= t])
                    ncs.append(n)
                    k += n
                    assert k == len(cs) or cs[k][1] > t
                for r in range(0, 1000):
                    nxs, k, credit, ok = [], 0, 0.0, True
                    for t in range(len(seq)):
                        if ncs[t] == 0:
                            n = XU0 if t < 15 else XU
                        else:
                            credit += r / 500.0
                            n = 1 if (credit >= 1.0 and ncs[t] == 1) else 0
                            credit -= n
                        n = min(n, len(xs) - k)
                        nxs.append(n)
                        k += n
                        ok = ok and (k == len(xs) or xs[k][1] > t)
                    if ok:
                        break
                for t, (kind, p, idx) in enumerate(seq):
                    res = self.run(kind, p, idx)
                    nc, nx = ncs[t], nxs[t]
                    nslot = 2 * nc + nx
                    nv = RC // 8

                    def dep_at(k):
                        i0 = (2 * k * nv) // (2 * nslot)
                        i1 = ((2 * k + 1) * nv) // (2 * nslot)
                        return jnp.concatenate([res[8 * i0:8 * i0 + 8], res[8 * i1:8 * i1 + 8]], axis=0)
                    for k in range(nx):
                        self.xprep(*xs.pop(0)[2], dep_at(k))
                    for k in range(nc):
                        self.cpair(*cs.pop(0)[2], [dep_at(nx + 2 * k), dep_at(nx + 2 * k + 1)])
                    if kind == 'm':
                        if p == nsc - 1:
                            if idx == 3:
                                self.out_dma(p, pl.ds(0, 256))
                            elif idx == 6:
                                self.out_dma(p, pl.ds(256, 256))
                        elif idx == 6:
                            self.out_dma(p, slice(None))
                assert not xs and not cs

            def carry(self, n):
                for c in range(NC):
                    h_ref[c, 0:16, :] = h_ref[c, n:n + 16, :]

        @pl.when(j == 0)
        def _():
            for g in groups:
                for cp in g:
                    cp.start()
            xbuf[R:R + 16, :] = jnp.zeros((16, D), bf16)
            for c in range(NC):
                h_ref[c, 0:8, :] = jnp.zeros((8, 128), f32)
            blk = Blk(xbuf, obuf, 0, {}, K - 1)

            def pw1_rows(c, lo=0, hi=X0, raw=True):
                xq = xbuf[lo:hi, :]
                a = jnp.dot(xq, w1tile(c, raw), preferred_element_type=f32)
                blk.attach(a, 3 * NP)
                b = jnp.dot(xq, w1tile(NC + c, raw), preferred_element_type=f32)
                blk.attach(b[0:hi - lo - 80], 2 * NP)
                g = a * (1.0 + jnp.tanh(0.5 * b))
                n = min(hi, X0 - 8) - lo
                h_ref[c, 8 + lo:8 + lo + n, :] = g[0:n]
                if hi == X0:
                    blk.todo.extend((q, c, p) for q in range(NP) for p in range(NPAIR))

            wait_group(0)
            pw1_rows(0, 0, XA)
            wait_group(1)
            pw1_rows(0, XA, X0, raw=False)
            dwf = dwraw[...].astype(f32) * 0.25
            for c in range(NC):
                for k in range(K):
                    dwb[c * K + k] = jnp.broadcast_to(dwf[k:k + 1, c * 128:(c + 1) * 128], (8, 128))
            wait_group(2)
            pw1_rows(1)
            wait_group(3)
            xb_copy(0).start()
            pw1_rows(2)
            pw1_rows(3)
            wait_group(4)
            blk.raw_w2 = True
            blk.extra = [(w, l, kl, i) for w in 'am' for l in range(2) for kl in range(2) for i in range(8)]
            blk.steady(NP, QP, list(range(NP)))
            assert not blk.extra
            blk.carry(TP)
            pltpu.make_async_copy(obuf.at[pl.ds(0, TP), :], o_hbm.at[pl.ds(0, TP), :], sem_out).start()

        @pl.when(j > 0)
        def _():
            i = j - 1
            xb_copy(i).wait()

            @pl.when(j < NB)
            def _():
                xb_copy(j).start()

            base = pl.multiple_of(TP + i * TB, 16)
            masks = {}
            last_flag = i == NB - 1
            if bnd_q == 0:
                last_flag = jnp.logical_or(last_flag, i == bnd_it - 1)
            else:
                masks[(bnd_q - 1, NPAIR - 1)] = ('last', i == bnd_it)
            masks[(QB - 1, NPAIR - 1)] = ('last', last_flag)
            masks[(bnd_q, 0)] = ('first', i == bnd_it)
            b = SBlk(xbuf.at[pl.ds(base, TB + 16), :], obuf.at[pl.ds(base, TB), :], base, masks)
            b.steady(QB // 2)
            b.carry(TB)

        @pl.when(j == NB)
        def _():
            pltpu.make_async_copy(o_hbm, o_hbm, sem_out).wait()

    opts = dict(dimension_semantics=("arbitrary",), vmem_limit_bytes=100 * 1024 * 1024)
    for name in ("disable_bounds_checks", "disable_semaphore_checks"):
        if hasattr(pltpu.CompilerParams, name):
            opts[name] = True

    out = pl.pallas_call(
        kernel,
        grid=(NB + 1,),
        in_specs=[pl.BlockSpec(memory_space=pl.ANY)] * 4,
        out_specs=pl.BlockSpec(memory_space=pl.ANY),
        out_shape=jax.ShapeDtypeStruct((R, D), x.dtype),
        scratch_shapes=[
            pltpu.VMEM((R + 16, D), bf16),
            pltpu.VMEM((2 * NC, D, 128), bf16),
            pltpu.VMEM((NC, D, 128), bf16),
            pltpu.VMEM((K, D), bf16),
            pltpu.VMEM((D // 2, 2 * D), u32),
            pltpu.VMEM((D // 2, D), u32),
            pltpu.VMEM((NC * K, 8, 128), f32),
            pltpu.VMEM((NC, HR, 128), f32),
            pltpu.VMEM((2, TP // 2, D), u32),
            pltpu.VMEM((R, D), bf16),
            pltpu.VMEM((7 * 128, 256), u32),
            pltpu.VMEM((7 * 128, 256), u32),
            pltpu.VMEM((2, QB // 2 * 5 * (RC // 2), 256), u32),
            pltpu.VMEM((2, QB * (RC // 2), D), u32),
            pltpu.VMEM((2, QB // 2 * 7 * (RC // 2), 256), u32),
            pltpu.VMEM((2, 4 * RC, D), f32),
            pltpu.SemaphoreType.DMA((5,)),
            pltpu.SemaphoreType.DMA,
            pltpu.SemaphoreType.DMA,
        ],
        compiler_params=pltpu.CompilerParams(**opts),
    )(x.reshape(R, D), w_pw1, dw, w_pw2)
    return out.reshape(B, T, D)
```

```python
import jax
import jax.numpy as jnp
import jax.experimental.pallas as pl
import jax.experimental.pallas.tpu as pltpu

RC = 80
NP = 6
XA = 176
QP = 12
QB = 44
XU0 = 7
LAGSC = 2
RESV = 21
LAG = 3
SDL = 2
SLAG = 2
XDL = 2
XU = 5
RING = 12
XST = 2
PSEQ = 'b3.b4.a3.a4.b5.a5.m0.m1.m2.m3.m4.m5'
DEBUG = 0
BORD = (0, 1, 2, 3, 1, 0, 3, 2)
IORD = (0, 2, 4, 1, 3)
T12 = ((0, 2), (1, 3))


@jax.jit
def pallas_standalone__conformer_conv_module__speech_kernel(x, w_pw1, dw, w_pw2):
    B, T, D = x.shape
    K = dw.shape[0]
    pad = K // 2
    R = B * T
    NC = D // 128
    NQ = R // RC
    NS = NQ // 2
    P0 = NP // 2
    assert T % (2 * RC) == 0 and pad <= 7 and NC == 4 and NP % 2 == 0
    f32, bf16, u32 = jnp.float32, jnp.bfloat16, jnp.uint32
    NPAIR = RC // 16
    RH = RC // 2
    X0 = NP * RC + 16
    TP = QP * RC
    TB = QB * RC
    NB = (R - TP) // TB
    assert TP + NB * TB == R and B == 2 and TP < T
    gq = (T - TP) // RC
    bnd_it, bnd_q = gq // QB, gq % QB
    HR = max(TP, TB) + 16
    X1 = TP + 8 * NB
    XN = TB - 8

    def kernel(x_hbm, w1_hbm, dw_hbm, w2_hbm, o_hbm,
               xbuf, w1raw, w2raw, dwraw, w1p, dwb, h_ref, obuf,
               wsa, wsm, xs_all, xr_all, ss_all, g_all, sem_in, sem_x, sem_out):
        j = pl.program_id(0)
        sub8 = jax.lax.broadcasted_iota(jnp.int32, (8, 128), 0)
        never = sub8 > j + 1000
        xs_ref, xr_ref, ss_ref, g_ref = xs_all.at[j % 2], xr_all.at[j % 2], ss_all.at[j % 2], g_all.at[j % 2]

        def pin(v, dep):
            if dep is None:
                return v
            if v.shape[0] == 8:
                return jnp.where(never, dep, v)
            return jnp.concatenate([jnp.where(never, dep, v[0:8]), v[8:]], axis=0)

        def st_packed(ref, r, t, v):
            ref[r:r + 8, t * 128:(t + 1) * 128] = pltpu.bitcast(v.astype(bf16), u32)

        def w1_copy(col, s):
            return pltpu.make_async_copy(w1_hbm.at[:, pl.ds(col * 128, 128)], w1raw.at[col], sem_in.at[s])

        def w2_copy(col, s):
            return pltpu.make_async_copy(w2_hbm.at[:, pl.ds(col * 128, 128)], w2raw.at[col], sem_in.at[s])

        def x_copy(lo, hi, s):
            return pltpu.make_async_copy(x_hbm.at[pl.ds(lo, hi - lo), :], xbuf.at[pl.ds(lo, hi - lo), :], sem_in.at[s])

        groups = [
            [x_copy(0, XA, 0), w1_copy(0, 0), w1_copy(NC, 0)],
            [x_copy(XA, X0, 1), pltpu.make_async_copy(dw_hbm, dwraw, sem_in.at[1])],
            [w1_copy(1, 2), w1_copy(NC + 1, 2)],
            [w1_copy(2, 3), w1_copy(NC + 2, 3), w1_copy(3, 3), w1_copy(NC + 3, 3)],
            [x_copy(X0, X1, 4)] + [w2_copy(n, 4) for n in range(NC)],
        ]

        def xb_copy(i):
            lo = X1 + i * XN
            if not isinstance(lo, int):
                lo = pl.multiple_of(lo, 8)
            return pltpu.make_async_copy(x_hbm.at[pl.ds(lo, XN), :], xbuf.at[pl.ds(lo, XN), :], sem_x)

        class ctx:
            xv, ov, obase, masks, direct = xbuf, obuf, 0, {}, ()

        def start_group(g):
            for cp in groups[g]:
                cp.start()

        def wait_group(g):
            for cp in groups[g]:
                cp.wait()

        def w1tile(col, raw=False):
            if raw:
                wt = w1raw[col]
                w1p[:, col * 128:(col + 1) * 128] = pltpu.bitcast(wt, u32)
                return wt
            return pltpu.bitcast(w1p[:, col * 128:(col + 1) * 128], bf16)

        def conv16(c, o, dep, ws):
            mode, flag = ctx.masks.get(o, (None, None))
            vs = []
            for s in range(K + 1):
                v = h_ref[c, pl.ds(8 + o + s - pad, 8, stride=2), :]
                rel = 2 * sub8 + (s - pad)
                if mode == 'last' and 14 + s - pad >= 16:
                    v = jnp.where(rel < jnp.where(flag, 16, 64), v, 0.0)
                elif mode == 'first' and s < pad:
                    v = jnp.where(rel >= jnp.where(flag, 0, -64), v, 0.0)
                vs.append(v)
            y0 = y1 = None
            for k in range(K):
                w = pin(ws[k], dep) if k == K - 1 else ws[k]
                t0, t1 = vs[k] * w, vs[k + 1] * w
                y0, y1 = (t0, t1) if y0 is None else (y0 + t0, y1 + t1)
            return y0 + y0 * jnp.tanh(y0), y1 + y1 * jnp.tanh(y1)

        sv = {}

        def cpair(p, l, i, half, deps):
            c = T12[half][l]
            ws = [dwb[c * K + k] for k in range(K)]
            out = [conv16(c, (2 * p + u) * RC + 16 * i, deps[u], ws) for u in range(2)]

            def put(n, a, b=None, sg=1):
                if b is not None:
                    a = [u + v if sg > 0 else u - v for u, v in zip(a, b)]
                r = ((p % RING) * 7 + n) * RH + 8 * i
                ss_ref[r:r + 8, l * 128:(l + 1) * 128] = pltpu.pack_elementwise(list(a), packed_dtype=bf16)
            if half == 0:
                s11, s21 = out
                put(2, s11)
                put(5, s21, s11, -1)
                sv[(p, l, i)] = out
            else:
                s11, s21 = sv.pop((p, l, i))
                s12, s22 = out
                put(0, s11, s22)
                put(1, s21, s22)
                put(3, s22)
                put(4, s11, s12)
                put(6, s12, s22, -1)

        def xprep(p, i, l, dep):
            def ld(q, t):
                r = q * RC + 8 + 16 * i
                cs = slice(t * 128, (t + 1) * 128)
                return jnp.concatenate([ctx.xv[r:r + 8, cs].astype(f32), ctx.xv[r + 8:r + 16, cs].astype(f32)], axis=0)
            q1, q2 = 2 * p, 2 * p + 1
            a11, a12, a21, a22 = pin(ld(q1, l), dep), ld(q1, l + 2), ld(q2, l), pin(ld(q2, l + 2), dep)
            for n, v in enumerate([a11 + a22, a21 + a22, a11 + a12, a21 - a11, a12 - a22]):
                st_packed(xs_ref, ((p % RING) * 5 + n) * RH + 8 * i, l, v)
            for u, t, v in [(0, l, a11), (0, l + 2, a12), (1, l, a21), (1, l + 2, a22)]:
                st_packed(xr_ref, ((p % RING) * 2 + u) * RH + 8 * i, t, v)

        def wprep(which, l, kl, i, dep):
            if which == 'a':
                raw, dst, kt, nt = w1raw, wsa, ((0, 1), (2, 3)), T12
            else:
                raw, dst, kt, nt = w2raw, wsm, T12, ((0, 2), (1, 3))

            def ld(kh, nh):
                r = kt[kh][kl] * 128 + 16 * i
                return raw[nt[nh][l], r:r + 16, :].astype(f32)
            b11, b12, b21, b22 = pin(ld(0, 0), dep), ld(0, 1), ld(1, 0), pin(ld(1, 1), dep)
            for n, v in enumerate([b11 + b22, b11, b12 - b22, b21 - b11, b22, b11 + b12, b21 + b22]):
                st_packed(dst, n * 128 + kl * 64 + 8 * i, l, v)

        def lhs(kind, p, n):
            pr = p % RING
            if kind == 'm':
                v = ss_ref[(pr * 7 + n) * RH:(pr * 7 + n + 1) * RH, :]
            elif n == 2:
                v = xr_ref[2 * pr * RH:(2 * pr + 1) * RH, 0:256]
            elif n == 3:
                v = xr_ref[(2 * pr + 1) * RH:(2 * pr + 2) * RH, 256:512]
            else:
                m = {0: 0, 1: 1, 4: 2, 5: 3, 6: 4}[n]
                v = xs_ref[(pr * 5 + m) * RH:(pr * 5 + m + 1) * RH, :]
            return pltpu.bitcast(v, bf16)

        def prod(kind, p, n, l):
            w = wsa if kind == 'a' else wsm
            wt = w[n * 128:(n + 1) * 128, :] if l is None else w[n * 128:(n + 1) * 128, l * 128:(l + 1) * 128]
            return jnp.dot(lhs(kind, p, n), pltpu.bitcast(wt, bf16), preferred_element_type=f32)

        def fin(kind, p, l, rh, ch, v):
            q = 2 * p + rh
            if kind == 'a':
                c = T12[ch][l]
                g = g_ref[(q % 4) * RC:(q % 4 + 1) * RC, c * 128:(c + 1) * 128]
                h_ref[c, 16 + q * RC:16 + (q + 1) * RC, :] = v * g
            else:
                c = 2 * l + ch
                ctx.ov[q * RC:(q + 1) * RC, c * 128:(c + 1) * 128] = v.astype(bf16)

        st = {}

        def run(kind, p, idx):
            if kind == 'b':
                u, c = idx % 2, BORD[idx]
                q = 2 * p + u
                if p in ctx.direct:
                    xq = ctx.xv[q * RC + 8:(q + 1) * RC + 8, :]
                else:
                    r = ((p % RING) * 2 + u) * RH
                    xq = pltpu.bitcast(xr_ref[r:r + RH, :], bf16)
                b = jnp.dot(xq, w1tile(NC + c), preferred_element_type=f32)
                g_ref[(q % 4) * RC:(q % 4 + 1) * RC, c * 128:(c + 1) * 128] = 1.0 + jnp.tanh(0.5 * b)
                return b
            l = 0 if idx < 3 else 1
            step = idx if idx < 3 else idx - 4
            if idx == 3:
                m6 = prod(kind, p, 5, None)
                fin(kind, p, 0, 1, 1, st.pop('t22') + m6[:, 0:128])
                st['t22'] = m6[:, 128:256]
                return m6[:, 0:128]
            if step == 0:
                m2, m4 = prod(kind, p, 1, l), prod(kind, p, 3, l)
                fin(kind, p, l, 1, 0, m2 + m4)
                st['t11'] = m4
                st['t22'] = m2 if l == 0 else st['t22'] - m2
                return m2
            if step == 1:
                m3, m5 = prod(kind, p, 2, l), prod(kind, p, 4, l)
                fin(kind, p, l, 0, 1, m3 + m5)
                st['t11'] = st['t11'] - m5
                st['t22'] = m3 - st['t22'] if l == 0 else st['t22'] + m3
                return m3
            m1, m7 = prod(kind, p, 0, l), prod(kind, p, 6, l)
            fin(kind, p, l, 0, 0, st.pop('t11') + m1 + m7)
            if l == 0:
                st['t22'] = st['t22'] + m1
            else:
                fin(kind, p, l, 1, 1, st.pop('t22') + m1)
            return m1

        def out_dma(p, cols):
            dst = ctx.obase + 2 * p * RC
            if not isinstance(dst, int):
                dst = pl.multiple_of(dst, 16)
            pltpu.make_async_copy(ctx.ov.at[pl.ds(2 * p * RC, 2 * RC), cols],
                                  o_hbm.at[pl.ds(dst, 2 * RC), cols], sem_out).start()

        def anchors(res, n):
            nv = res.shape[0] // 8
            ks = [((2 * k + 1) * nv) // (2 * n) for k in range(n)]
            return [res[8 * k:8 * k + 8] for k in ks]

        def pipeline(groups_, p0, ns, todo, with_w, split_last):
            seq = [(kind, p, i) for kind, p in groups_ for i in range(8 if kind == 'b' else 7)]
            pos = {it: t for t, it in enumerate(seq)}
            sm, cs = [], []
            if with_w:
                for w, dl in (('a', pos[('a', p0, 0)]), ('m', pos[('m', 0, 0)])):
                    sm += [(0, dl - XDL, wprep, (w, l, kl, i)) for l in range(2) for kl in range(2) for i in range(8)]
            for p in range(p0, ns):
                dl = pos[('a' if p in ctx.direct else 'b', p, 0)] - XDL
                av = pos[('a', p - RING, 6)] + 1 if p - RING >= p0 else 0
                sm += [(av, dl, xprep, (p, i, l)) for i in range(NPAIR) for l in range(2)]
            sm.sort(key=lambda it: it[1])
            cs += [(0, pos[('m', it[0], 0)] - SDL, it) for it in todo]
            for p in range(p0, ns):
                for l in range(2):
                    for i in IORD:
                        for half in range(2):
                            av = pos[('a', p, (2 + half) if l == 0 else 6)] + SLAG
                            cs.append((av, pos[('m', p, 0)] - SDL, (p, l, i, half)))

            def plan(rate):
                out, kc, ks, credit, worst = [], 0, 0, 0.0, 0
                for t in range(len(seq)):
                    c_slack = min([it[1] - t - i for i, it in enumerate(cs[kc:kc + 80])], default=99)
                    s_slack = min([it[1] - t - i // XU for i, it in enumerate(sm[ks:ks + 80])], default=99)
                    nc = len([it for it in cs[kc:kc + (2 if c_slack < 0 else 1)] if it[0] <= t])
                    if s_slack <= 0 and c_slack > 0:
                        nc = 0
                    if nc == 0 or s_slack <= 0:
                        nx = XU0 if (t < 15 and nc == 0) else XU
                    else:
                        credit = min(credit + rate, 1.5)
                        nx = 1 if credit >= 1.0 else 0
                    nx = len([it for it in sm[ks:ks + nx] if it[0] <= t])
                    if nc:
                        credit -= min(nx, 1)
                    worst += (nc > 1) + (nc > 0 and nx > 1)
                    out.append((nc, nx))
                    kc += nc
                    ks += nx
                    assert (kc == len(cs) or cs[kc][1] > t) and (ks == len(sm) or sm[ks][1] > t)
                return worst, out
            plans = [plan(r / 100.0) for r in range(0, 101, 2)]
            best = min(w for w, o in plans)
            sched = next(o for w, o in plans if w == best)
            if DEBUG:
                print("worst", best, ''.join('%d%d ' % o for o in sched[:120]))

            for t, (kind, p, idx) in enumerate(seq):
                res = run(kind, p, idx)
                nc, nx = sched[t]
                if nc + nx:
                    an = anchors(res, 2 * nc + nx)
                    for k in range(nx):
                        it = sm.pop(0)
                        it[2](*it[3], an[k])
                    for k in range(nc):
                        cpair(*cs.pop(0)[2], an[nx + 2 * k:nx + 2 * k + 2])
                if kind == 'm' and split_last:
                    if p == ns - 1:
                        if idx == 3:
                            out_dma(p, pl.ds(0, 256))
                        elif idx == 6:
                            out_dma(p, pl.ds(256, 256))
                    elif idx == 6:
                        out_dma(p, slice(None))
            assert not sm and not cs
            n = 2 * ns * RC
            for c in range(NC):
                h_ref[c, 0:16, :] = h_ref[c, n:n + 16, :]

        @pl.when(j == 0)
        def _():
            for g in range(5):
                start_group(g)
            xbuf[R:R + 16, :] = jnp.zeros((16, D), bf16)
            for c in range(NC):
                h_ref[c, 0:8, :] = jnp.zeros((8, 128), f32)

            todo = []

            def attach(res, n):
                n = min(n, len(todo))
                if n:
                    an = anchors(res, 2 * n)
                    for k in range(n):
                        cpair(*todo.pop(0), an[2 * k:2 * k + 2])

            def pw1_rows(c, lo=0, hi=X0, raw=True):
                xq = xbuf[lo:hi, :]
                a = jnp.dot(xq, w1tile(c, raw), preferred_element_type=f32)
                attach(a, 3 * P0)
                b = jnp.dot(xq, w1tile(NC + c, raw), preferred_element_type=f32)
                attach(b[0:hi - lo - 80], 2 * P0)
                g = a * (1.0 + jnp.tanh(0.5 * b))
                n = min(hi, X0 - 8) - lo
                h_ref[c, 8 + lo:8 + lo + n, :] = g[0:n]
                if hi == X0:
                    todo.extend((p, c // 2, i, c % 2) for p in range(P0) for i in IORD)

            wait_group(0)
            pw1_rows(0, 0, XA)
            wait_group(1)
            pw1_rows(0, XA, X0, raw=False)
            dwf = dwraw[...].astype(f32) * 0.25
            for c in range(NC):
                for k in range(K):
                    dwb[c * K + k] = jnp.broadcast_to(dwf[k:k + 1, c * 128:(c + 1) * 128], (8, 128))
            wait_group(2)
            if XST == 2:
                xb_copy(0).start()
            pw1_rows(1)
            wait_group(3)
            if XST == 3:
                xb_copy(0).start()
            pw1_rows(2)
            pw1_rows(3)
            wait_group(4)

            ctx.direct = (P0, P0 + 1)
            pipeline([(s[0], int(s[1:])) for s in PSEQ.split('.')], P0, QP // 2, todo, True, False)
            pltpu.make_async_copy(obuf.at[pl.ds(0, TP), :], o_hbm.at[pl.ds(0, TP), :], sem_out).start()

        @pl.when(j > 0)
        def _():
            i = j - 1
            xb_copy(i).wait()

            @pl.when(j < NB)
            def _():
                xb_copy(j).start()

            base = pl.multiple_of(TP + i * TB, 16)
            masks = {}
            last_flag = i == NB - 1
            if bnd_q == 0:
                last_flag = jnp.logical_or(last_flag, i == bnd_it - 1)
            else:
                masks[bnd_q * RC - 16] = ('last', i == bnd_it)
            masks[TB - 16] = ('last', last_flag)
            masks[bnd_q * RC] = ('first', i == bnd_it)
            ctx.xv, ctx.ov = xbuf.at[pl.ds(base, TB + 16), :], obuf.at[pl.ds(base, TB), :]
            ctx.obase, ctx.masks, ctx.direct = base, masks, (0,)
            ns = QB // 2
            gs = []
            for p in range(ns):
                gs += [('b', p), ('a', p)]
                if p >= LAGSC and 7 * (ns - 1 - (p - LAGSC)) > RESV:
                    gs.append(('m', p - LAGSC))
            gs += [('m', p) for p in range(ns) if ('m', p) not in gs]
            pipeline(gs, 0, ns, [], False, True)

        @pl.when(j == NB)
        def _():
            pltpu.make_async_copy(o_hbm, o_hbm, sem_out).wait()

    opts = dict(dimension_semantics=("arbitrary",), vmem_limit_bytes=100 * 1024 * 1024)
    for name in ("disable_bounds_checks", "disable_semaphore_checks"):
        if hasattr(pltpu.CompilerParams, name):
            opts[name] = True

    out = pl.pallas_call(
        kernel,
        grid=(NB + 1,),
        in_specs=[pl.BlockSpec(memory_space=pl.ANY)] * 4,
        out_specs=pl.BlockSpec(memory_space=pl.ANY),
        out_shape=jax.ShapeDtypeStruct((R, D), x.dtype),
        scratch_shapes=[
            pltpu.VMEM((R + 16, D), bf16),
            pltpu.VMEM((2 * NC, D, 128), bf16),
            pltpu.VMEM((NC, D, 128), bf16),
            pltpu.VMEM((K, D), bf16),
            pltpu.VMEM((D // 2, 2 * D), u32),
            pltpu.VMEM((NC * K, 8, 128), f32),
            pltpu.VMEM((NC, HR, 128), f32),
            pltpu.VMEM((R, D), bf16),
            pltpu.VMEM((7 * 128, 256), u32),
            pltpu.VMEM((7 * 128, 256), u32),
            pltpu.VMEM((2, RING * 5 * RH, 256), u32),
            pltpu.VMEM((2, RING * 2 * RH, D), u32),
            pltpu.VMEM((2, RING * 7 * RH, 256), u32),
            pltpu.VMEM((2, 4 * RC, D), f32),
            pltpu.SemaphoreType.DMA((5,)),
            pltpu.SemaphoreType.DMA,
            pltpu.SemaphoreType.DMA,
        ],
        compiler_params=pltpu.CompilerParams(**opts),
    )(x.reshape(R, D), w_pw1, dw, w_pw2)
    return out.reshape(B, T, D)
```

```python
import jax
import jax.numpy as jnp
import jax.experimental.pallas as pl
import jax.experimental.pallas.tpu as pltpu

RC = 80
NP = 6
XA = 176
QP = 12
QB = 44
XU0 = 7
LAGSC = 2
RESV = 35
LAG = 3
SDL = 2
SLAG = 2
XDL = 2
XU = 5
RING = 12
QRING = 3
XRR = 8
FMAX = 16
ANC = 1
ANM = 1
BCOST = 60
CCAP = 35
NMAX = 3
FSKIP = 4
XEARLY = 0
XPOS = (1, 4, 7, 10, 13)
LAGQ = 1
SA = ((1, 0, 0, 1), (0, 0, 1, 1), (1, 0, 0, 0), (0, 0, 0, 1), (1, 1, 0, 0), (-1, 0, 1, 0), (0, 1, 0, -1))
SB = ((1, 0, 0, 1), (1, 0, 0, 0), (0, 1, 0, -1), (-1, 0, 1, 0), (0, 0, 0, 1), (1, 1, 0, 0), (0, 0, 1, 1))
MORD = (1, 3, 2, 4, 0, 6, 5)
XST = 2
PSEQ = 'b3.b4.a3.a4.b5.a5.m0.m1.m2.m3.m4.m5'
DEBUG = 0
BORD = (0, 1, 2, 3, 1, 0, 3, 2)
IORD = (0, 2, 4, 1, 3)
T12 = ((0, 2), (1, 3))


@jax.jit
def pallas_standalone__conformer_conv_module__speech_kernel(x, w_pw1, dw, w_pw2):
    B, T, D = x.shape
    K = dw.shape[0]
    pad = K // 2
    R = B * T
    NC = D // 128
    NQ = R // RC
    NS = NQ // 2
    P0 = NP // 2
    assert T % (2 * RC) == 0 and pad <= 7 and NC == 4 and NP % 2 == 0
    f32, bf16, u32 = jnp.float32, jnp.bfloat16, jnp.uint32
    NPAIR = RC // 16
    RH = RC // 2
    X0 = NP * RC + 16
    TP = QP * RC
    TB = QB * RC
    NB = (R - TP) // TB
    assert TP + NB * TB == R and B == 2 and TP < T
    gq = (T - TP) // RC
    bnd_it, bnd_q = gq // QB, gq % QB
    HR = max(TP, TB) + 16
    X1 = TP + 8 * NB
    XN = TB - 8

    def kernel(x_hbm, w1_hbm, dw_hbm, w2_hbm, o_hbm,
               xbuf, w1raw, w2raw, dwraw, w1p, dwb, h_ref, obuf,
               wsa, wsm, xs_all, xr_all, ss_all, g_all, wsa2, x2_all, t_all, sem_in, sem_x, sem_out):
        j = pl.program_id(0)
        sub8 = jax.lax.broadcasted_iota(jnp.int32, (8, 128), 0)
        never = sub8 > j + 1000
        xs_ref, xr_ref, ss_ref, g_ref = xs_all.at[j % 2], xr_all.at[j % 2], ss_all.at[j % 2], g_all.at[j % 2]

        def pin(v, dep):
            if dep is None:
                return v
            if v.shape[0] == 8:
                return jnp.where(never, dep, v)
            return jnp.concatenate([jnp.where(never, dep, v[0:8]), v[8:]], axis=0)

        def st_packed(ref, r, t, v):
            ref[r:r + 8, t * 128:(t + 1) * 128] = pltpu.bitcast(v.astype(bf16), u32)

        def w1_copy(col, s):
            return pltpu.make_async_copy(w1_hbm.at[:, pl.ds(col * 128, 128)], w1raw.at[col], sem_in.at[s])

        def w2_copy(col, s):
            return pltpu.make_async_copy(w2_hbm.at[:, pl.ds(col * 128, 128)], w2raw.at[col], sem_in.at[s])

        def x_copy(lo, hi, s):
            return pltpu.make_async_copy(x_hbm.at[pl.ds(lo, hi - lo), :], xbuf.at[pl.ds(lo, hi - lo), :], sem_in.at[s])

        groups = [
            [x_copy(0, XA, 0), w1_copy(0, 0), w1_copy(NC, 0)],
            [x_copy(XA, X0, 1), pltpu.make_async_copy(dw_hbm, dwraw, sem_in.at[1])],
            [w1_copy(1, 2), w1_copy(NC + 1, 2)],
            [w1_copy(2, 3), w1_copy(NC + 2, 3), w1_copy(3, 3), w1_copy(NC + 3, 3)],
            [x_copy(X0, X1, 4)] + [w2_copy(n, 4) for n in range(NC)],
        ]

        def xb_copy(i):
            lo = X1 + i * XN
            if not isinstance(lo, int):
                lo = pl.multiple_of(lo, 8)
            return pltpu.make_async_copy(x_hbm.at[pl.ds(lo, XN), :], xbuf.at[pl.ds(lo, XN), :], sem_x)

        class ctx:
            xv, ov, obase, masks, direct, xrr = xbuf, obuf, 0, {}, (), 2 * RING

        def start_group(g):
            for cp in groups[g]:
                cp.start()

        def wait_group(g):
            for cp in groups[g]:
                cp.wait()

        def w1tile(col, raw=False):
            if raw:
                wt = w1raw[col]
                w1p[:, col * 128:(col + 1) * 128] = pltpu.bitcast(wt, u32)
                return wt
            return pltpu.bitcast(w1p[:, col * 128:(col + 1) * 128], bf16)

        def conv16(c, o, dep, ws):
            mode, flag = ctx.masks.get(o, (None, None))
            vs = []
            for s in range(K + 1):
                v = h_ref[c, pl.ds(8 + o + s - pad, 8, stride=2), :]
                rel = 2 * sub8 + (s - pad)
                if mode == 'last' and 14 + s - pad >= 16:
                    v = jnp.where(rel < jnp.where(flag, 16, 64), v, 0.0)
                elif mode == 'first' and s < pad:
                    v = jnp.where(rel >= jnp.where(flag, 0, -64), v, 0.0)
                vs.append(v)
            y0 = y1 = None
            for k in range(K):
                w = pin(ws[k], dep) if k == K - 1 else ws[k]
                t0, t1 = vs[k] * w, vs[k + 1] * w
                y0, y1 = (t0, t1) if y0 is None else (y0 + t0, y1 + t1)
            return y0 + y0 * jnp.tanh(y0), y1 + y1 * jnp.tanh(y1)

        sv = {}

        def cpair(p, l, i, half, deps):
            for u in range(2):
                c16(p, l, i, half, u, deps[u])

        def c16(p, l, i, half, u, dep):
            c = T12[half][l]
            ws = [dwb[c * K + k] for k in range(K)]
            y = conv16(c, (2 * p + u) * RC + 16 * i, dep, ws)
            if u == 0:
                sv[(p, l, i, half)] = y
                if half == 0:
                    r = ((p % RING) * 7 + 2) * RH + 8 * i
                    ss_ref[r:r + 8, l * 128:(l + 1) * 128] = pltpu.pack_elementwise(list(y), packed_dtype=bf16)
                else:
                    s11 = sv[(p, l, i)][0]
                    r = ((p % RING) * 7 + 4) * RH + 8 * i
                    ss_ref[r:r + 8, l * 128:(l + 1) * 128] = pltpu.pack_elementwise(
                        [s11[0] + y[0], s11[1] + y[1]], packed_dtype=bf16)
                return
            out = [sv.pop((p, l, i, half)), y]

            def put(n, a, b=None, sg=1):
                if b is not None:
                    a = [u + v if sg > 0 else u - v for u, v in zip(a, b)]
                r = ((p % RING) * 7 + n) * RH + 8 * i
                ss_ref[r:r + 8, l * 128:(l + 1) * 128] = pltpu.pack_elementwise(list(a), packed_dtype=bf16)
            if half == 0:
                s11, s21 = out
                put(5, s21, s11, -1)
                sv[(p, l, i)] = out
            else:
                s11, s21 = sv.pop((p, l, i))
                s12, s22 = out
                put(0, s11, s22)
                put(1, s21, s22)
                put(3, s22)
                put(6, s12, s22, -1)

        def xprep(p, i, l, dep):
            def ld(q, t):
                r = q * RC + 8 + 16 * i
                cs = slice(t * 128, (t + 1) * 128)
                return jnp.concatenate([ctx.xv[r:r + 8, cs].astype(f32), ctx.xv[r + 8:r + 16, cs].astype(f32)], axis=0)
            q1, q2 = 2 * p, 2 * p + 1
            a11, a12, a21, a22 = pin(ld(q1, l), dep), ld(q1, l + 2), ld(q2, l), pin(ld(q2, l + 2), dep)
            for n, v in enumerate([a11 + a22, a21 + a22, a11 + a12, a21 - a11, a12 - a22]):
                st_packed(xs_ref, ((p % RING) * 5 + n) * RH + 8 * i, l, v)
            for u, t, v in [(0, l, a11), (0, l + 2, a12), (1, l, a21), (1, l + 2, a22)]:
                st_packed(xr_ref, ((p % RING) * 2 + u) * RH + 8 * i, t, v)

        def wprep(which, l, kl, i, dep):
            if which == 'a':
                raw, dst, kt, nt = w1raw, wsa, ((0, 1), (2, 3)), T12
            else:
                raw, dst, kt, nt = w2raw, wsm, T12, ((0, 2), (1, 3))

            def ld(kh, nh):
                r = kt[kh][kl] * 128 + 16 * i
                return raw[nt[nh][l], r:r + 16, :].astype(f32)
            b11, b12, b21, b22 = pin(ld(0, 0), dep), ld(0, 1), ld(1, 0), pin(ld(1, 1), dep)
            for n, v in enumerate([b11 + b22, b11, b12 - b22, b21 - b11, b22, b11 + b12, b21 + b22]):
                st_packed(dst, n * 128 + kl * 64 + 8 * i, l, v)

        def comb(coef, vals):
            pos_ = [v for s, v in zip(coef, vals) if s > 0]
            neg_ = [v for s, v in zip(coef, vals) if s < 0]
            acc = pos_[0]
            for v in pos_[1:]:
                acc = acc + v
            for v in neg_:
                acc = acc - v
            return acc

        def leaves(S, X, deps, emit):
            if deps is not None:
                for k, (o, n) in enumerate(((3, 3), (3, 0), (0, 3), (0, 0))):
                    X[o][n] = pin(X[o][n], deps[k])
            for I in (3, 1, 6, 2, 0, 4, 5):
                O = [comb(S[I], [X[o][n] for o in range(4)]) for n in range(4)]
                for J in (3, 1, 6, 2, 0, 4, 5):
                    emit(I, J, comb(S[J], O))

        x2_ref, t_ref = x2_all.at[j % 2], t_all.at[j % 2]

        def xmega(Q, i, deps):
            def ld(o, n):
                q = 4 * Q + 2 * (o // 2) + n // 2
                t = 2 * (o % 2) + n % 2
                r = q * RC + 8 + 16 * i
                cs = slice(t * 128, (t + 1) * 128)
                return jnp.concatenate([ctx.xv[r:r + 8, cs].astype(f32), ctx.xv[r + 8:r + 16, cs].astype(f32)], axis=0)
            X = [[ld(o, n) for n in range(4)] for o in range(4)]

            def emit(I, J, v):
                if not (I in (2, 3) and J in (2, 3)):
                    st_packed(x2_ref, ((Q % QRING) * 25 + (7 * I + J) // 2) * RH + 8 * i, (7 * I + J) % 2, v)
            leaves(SA, X, deps, emit)

        def xraw(Q):
            for q in range(4 * Q, 4 * Q + 4):
                r = (q % XRR) * RH
                xr_ref[r:r + RH, :] = pltpu.bitcast(ctx.xv[q * RC + 8:(q + 1) * RC + 8, :], u32)

        def wmega(i, deps):
            def ld(o, n):
                r = (2 * (o // 2) + n // 2) * 128 + 16 * i
                return w1raw[2 * (o % 2) + n % 2, r:r + 16, :].astype(f32)
            X = [[ld(o, n) for n in range(4)] for o in range(4)]
            leaves(SB, X, deps, lambda I, J, v: st_packed(wsa2, (7 * I + J) // 2 * 64 + 8 * i, (7 * I + J) % 2, v))

        slot = [0]
        inner, outer = {}, {}

        def keep(name, v):
            slot[0] = (slot[0] + 1) % 32
            t_ref[slot[0] * RC:(slot[0] + 1) * RC, :] = v
            outer[name] = slot[0]

        def get(name):
            s = outer[name]
            return t_ref[s * RC:(s + 1) * RC, :]

        def fin2(Q, o, n, v):
            q = 4 * Q + 2 * (o // 2) + n // 2
            c = 2 * (o % 2) + n % 2
            g = g_ref[(q % 4) * RC:(q % 4 + 1) * RC, c * 128:(c + 1) * 128]
            h_ref[c, 16 + q * RC:16 + (q + 1) * RC, :] = v * g

        def outer_step(Q, I, n, m):
            if I == 1:
                keep(('m2', n), m)
            elif I == 3:
                fin2(Q, 2, n, get(('m2', n)) + m)
                keep(('t11', n), m)
            elif I == 2:
                keep(('m3', n), m)
                keep(('t22', n), m - get(('m2', n)))
            elif I == 4:
                fin2(Q, 1, n, get(('m3', n)) + m)
                keep(('t11', n), get(('t11', n)) - m)
            elif I == 0:
                keep(('t11', n), get(('t11', n)) + m)
                keep(('t22', n), get(('t22', n)) + m)
            elif I == 6:
                fin2(Q, 0, n, get(('t11', n)) + m)
            else:
                fin2(Q, 3, n, get(('t22', n)) + m)

        def leaf_job(Q, I, J):
            e = 7 * I + J
            if I in (2, 3) and J in (2, 3):
                o, n = 3 * (I - 2), 3 * (J - 2)
                q = 4 * Q + 2 * (o // 2) + n // 2
                t = 2 * (o % 2) + n % 2
                r = (q % XRR) * RH
                a = xr_ref[r:r + RH, t * 128:(t + 1) * 128]
            else:
                r = ((Q % QRING) * 25 + e // 2) * RH
                a = x2_ref[r:r + RH, (e % 2) * 128:(e % 2 + 1) * 128]
            w = wsa2[e // 2 * 64:(e // 2 + 1) * 64, (e % 2) * 128:(e % 2 + 1) * 128]
            m = jnp.dot(pltpu.bitcast(a, bf16), pltpu.bitcast(w, bf16), preferred_element_type=f32)
            s = inner
            if J == 1:
                s['m2'] = m
            elif J == 3:
                outer_step(Q, I, 2, s['m2'] + m)
                s['t11'] = m
            elif J == 2:
                s['m3'] = m
                s['t22'] = m - s.pop('m2')
            elif J == 4:
                outer_step(Q, I, 1, s.pop('m3') + m)
                s['t11'] = s['t11'] - m
            elif J == 0:
                s['t11'] = s['t11'] + m
                s['t22'] = s['t22'] + m
            elif J == 6:
                outer_step(Q, I, 0, s.pop('t11') + m)
            else:
                outer_step(Q, I, 3, s.pop('t22') + m)
            return m

        def lhs(kind, p, n):
            pr = p % RING
            if kind == 'm':
                v = ss_ref[(pr * 7 + n) * RH:(pr * 7 + n + 1) * RH, :]
            elif n == 2:
                v = xr_ref[2 * pr * RH:(2 * pr + 1) * RH, 0:256]
            elif n == 3:
                v = xr_ref[(2 * pr + 1) * RH:(2 * pr + 2) * RH, 256:512]
            else:
                m = {0: 0, 1: 1, 4: 2, 5: 3, 6: 4}[n]
                v = xs_ref[(pr * 5 + m) * RH:(pr * 5 + m + 1) * RH, :]
            return pltpu.bitcast(v, bf16)

        def prod(kind, p, n, l):
            w = wsa if kind == 'a' else wsm
            wt = w[n * 128:(n + 1) * 128, :] if l is None else w[n * 128:(n + 1) * 128, l * 128:(l + 1) * 128]
            return jnp.dot(lhs(kind, p, n), pltpu.bitcast(wt, bf16), preferred_element_type=f32)

        def fin(kind, p, l, rh, ch, v):
            q = 2 * p + rh
            if kind == 'a':
                c = T12[ch][l]
                g = g_ref[(q % 4) * RC:(q % 4 + 1) * RC, c * 128:(c + 1) * 128]
                h_ref[c, 16 + q * RC:16 + (q + 1) * RC, :] = v * g
            else:
                c = 2 * l + ch
                ctx.ov[q * RC:(q + 1) * RC, c * 128:(c + 1) * 128] = v.astype(bf16)

        st = {}

        def run(kind, p, idx):
            if kind == 'b':
                u, c = idx % 2, BORD[idx]
                q = 2 * p + u
                if p in ctx.direct:
                    xq = ctx.xv[q * RC + 8:(q + 1) * RC + 8, :]
                else:
                    r = (q % ctx.xrr) * RH
                    xq = pltpu.bitcast(xr_ref[r:r + RH, :], bf16)
                b = jnp.dot(xq, w1tile(NC + c), preferred_element_type=f32)
                g_ref[(q % 4) * RC:(q % 4 + 1) * RC, c * 128:(c + 1) * 128] = 1.0 + jnp.tanh(0.5 * b)
                return b
            l = 0 if idx < 3 else 1
            step = idx if idx < 3 else idx - 4
            if idx == 3:
                m6 = prod(kind, p, 5, None)
                fin(kind, p, 0, 1, 1, st.pop('t22') + m6[:, 0:128])
                st['t22'] = m6[:, 128:256]
                return m6[:, 128 * ANM:128 * ANM + 128]
            if step == 0:
                m2, m4 = prod(kind, p, 1, l), prod(kind, p, 3, l)
                fin(kind, p, l, 1, 0, m2 + m4)
                st['t11'] = m4
                st['t22'] = m2 if l == 0 else st['t22'] - m2
                return m4 if ANM else m2
            if step == 1:
                m3, m5 = prod(kind, p, 2, l), prod(kind, p, 4, l)
                fin(kind, p, l, 0, 1, m3 + m5)
                st['t11'] = st['t11'] - m5
                st['t22'] = m3 - st['t22'] if l == 0 else st['t22'] + m3
                return m5 if ANM else m3
            m1, m7 = prod(kind, p, 0, l), prod(kind, p, 6, l)
            fin(kind, p, l, 0, 0, st.pop('t11') + m1 + m7)
            if l == 0:
                st['t22'] = st['t22'] + m1
            else:
                fin(kind, p, l, 1, 1, st.pop('t22') + m1)
            return m7 if ANM else m1

        def out_dma(p, cols):
            dst = ctx.obase + 2 * p * RC
            if not isinstance(dst, int):
                dst = pl.multiple_of(dst, 16)
            pltpu.make_async_copy(ctx.ov.at[pl.ds(2 * p * RC, 2 * RC), cols],
                                  o_hbm.at[pl.ds(dst, 2 * RC), cols], sem_out).start()

        def anchors(res, n):
            nv = res.shape[0] // 8
            ks = [((2 * k + 1) * nv) // (2 * n) for k in range(n)]
            return [res[8 * k:8 * k + 8] for k in ks]

        def pipeline(groups_, p0, ns, todo, with_w, split_last):
            seq = [(kind, p, i) for kind, p in groups_ for i in range(8 if kind == 'b' else 7)]
            pos = {it: t for t, it in enumerate(seq)}
            sm, cs = [], []
            if with_w:
                for w, dl in (('a', pos[('a', p0, 0)]), ('m', pos[('m', 0, 0)])):
                    sm += [(0, dl - XDL, wprep, (w, l, kl, i)) for l in range(2) for kl in range(2) for i in range(8)]
            for p in range(p0, ns):
                dl = pos[('a' if p in ctx.direct else 'b', p, 0)] - XDL
                av = pos[('a', p - RING, 6)] + 1 if p - RING >= p0 else 0
                sm += [(av, dl, xprep, (p, i, l)) for i in range(NPAIR) for l in range(2)]
            sm.sort(key=lambda it: it[1])
            cs += [(0, pos[('m', it[0], 0)] - SDL, it) for it in todo]
            for p in range(p0, ns):
                for l in range(2):
                    for i in IORD:
                        for half in range(2):
                            av = pos[('a', p, (2 + half) if l == 0 else 6)] + SLAG
                            cs.append((av, pos[('m', p, 0)] - SDL, (p, l, i, half)))

            def plan(rate):
                out, kc, ks, credit, worst = [], 0, 0, 0.0, 0
                for t in range(len(seq)):
                    c_slack = min([it[1] - t - i for i, it in enumerate(cs[kc:kc + 80])], default=99)
                    s_slack = min([it[1] - t - i // XU for i, it in enumerate(sm[ks:ks + 80])], default=99)
                    nc = len([it for it in cs[kc:kc + (2 if c_slack < 0 else 1)] if it[0] <= t])
                    if s_slack <= 0 and c_slack > 0:
                        nc = 0
                    if nc == 0 or s_slack <= 0:
                        nx = XU0 if (t < 15 and nc == 0) else XU
                    else:
                        credit = min(credit + rate, 1.5)
                        nx = 1 if credit >= 1.0 else 0
                    nx = len([it for it in sm[ks:ks + nx] if it[0] <= t])
                    if nc:
                        credit -= min(nx, 1)
                    worst += (nc > 1) + (nc > 0 and nx > 1)
                    out.append((nc, nx))
                    kc += nc
                    ks += nx
                    assert (kc == len(cs) or cs[kc][1] > t) and (ks == len(sm) or sm[ks][1] > t)
                return worst, out
            plans = [plan(r / 100.0) for r in range(0, 101, 2)]
            best = min(w for w, o in plans)
            sched = next(o for w, o in plans if w == best)
            if DEBUG:
                print("worst", best, ''.join('%d%d ' % o for o in sched[:120]))

            for t, (kind, p, idx) in enumerate(seq):
                res = run(kind, p, idx)
                nc, nx = sched[t]
                if with_w and t >= len(seq) - 9 and t < len(seq) - 1:
                    wmega(t - (len(seq) - 9), anchors(res[0:RC - XEARLY], 4))
                if nc + nx:
                    an = anchors(res, 2 * nc + nx)
                    for k in range(nx):
                        it = sm.pop(0)
                        it[2](*it[3], an[k])
                    for k in range(nc):
                        cpair(*cs.pop(0)[2], an[nx + 2 * k:nx + 2 * k + 2])
                if kind == 'm' and split_last:
                    if p == ns - 1:
                        if idx == 3:
                            out_dma(p, pl.ds(0, 256))
                        elif idx == 6:
                            out_dma(p, pl.ds(256, 256))
                    elif idx == 6:
                        out_dma(p, slice(None))
            assert not sm and not cs
            n = 2 * ns * RC
            for c in range(NC):
                h_ref[c, 0:16, :] = h_ref[c, n:n + 16, :]

        def pipeline2(nq):
            jobs = [(Q, I, J) for Q in range(nq) for I in MORD for J in MORD]
            ap = [jobs[k:k + 4] for k in range(0, len(jobs), 4)]
            ns = 2 * nq
            seq, mdone = [], 0
            for Q in range(nq):
                seq += [('b', 2 * Q + k // 8, k % 8) for k in range(16)]
                seq += [('A', k, 0) for k in range(len(ap)) if ap[k][0][0] == Q]
                for p in (2 * (Q - LAGQ), 2 * (Q - LAGQ) + 1):
                    if p >= 0 and 7 * (ns - 1 - p) > RESV:
                        seq += [('m', p, i) for i in range(7)]
                        mdone = p + 1
            seq += [('m', p, i) for p in range(mdone, ns) for i in range(7)]
            pos = {it: t for t, it in enumerate(seq)}
            jpos = {jb: pos[('A', k, 0)] for k, js in enumerate(ap) for jb in js}
            lastp = {2: 3, 1: 4, 0: 6, 3: 5}
            tfin = {}
            for Q in range(nq):
                for o in range(4):
                    for n in range(4):
                        tfin[(4 * Q + 2 * (o // 2) + n // 2, 2 * (o % 2) + n % 2)] = jpos[(Q, lastp[o], lastp[n])]
            quads = []
            for p in range(ns):
                for l in range(2):
                    for i in IORD:
                        qs = [2 * p, 2 * p + 1] + ([2 * p - 1] if i == 0 and p > 0 else [])
                        av = max(tfin[(q, 2 * l + h)] for q in qs for h in range(2)) + SLAG
                        quads.append((av, pos[('m', p, 0)] - SDL, p, l, i))
            quads.sort(key=lambda it: it[0])
            cs = [(av, dl, (p, l, i, half, u)) for av, dl, p, l, i in quads for half in range(2) for u in range(2)]
            xat = {}
            free = [t for t in range(FMAX) if t % FSKIP != FSKIP - 1]
            for Q in range(nq):
                for i in range(NPAIR):
                    if free and Q < QRING:
                        t = free.pop(0)
                    else:
                        t = pos[('b', 2 * (Q - 1), 0)] + XPOS[i]
                    assert t <= jpos[(Q, MORD[0], MORD[0])] - XDL and t not in xat
                    assert Q < QRING or t > jpos[(Q - QRING, MORD[6], MORD[6])]
                    xat[t] = (Q, i)

            icost = (20, 0, 10, 10, 20, 10, 10)
            ocost = (20, 0, 10, 20, 30, 20, 20)
            own = []
            for t, (kind, p, idx) in enumerate(seq):
                if kind == 'b':
                    v = BCOST
                elif kind == 'm':
                    v = (40, 60, 60, 40, 50, 60, 70)[idx]
                else:
                    v = sum(icost[J] + (ocost[I] if J in (3, 4, 5, 6) else 0) for _, I, J in ap[p])
                own.append(v + (191 if t in xat else 0))

            def plan(rate):
                out, kc, credit = [], 0, 0.0
                for t in range(len(seq)):
                    credit = min(credit, CCAP) + rate - own[t]
                    n = max(0, min(NMAX, int(credit / 69.0 + 0.5)))
                    n = next((k for k, it in enumerate(cs[kc:kc + n]) if it[0] > t), min(n, len(cs) - kc))
                    credit -= 69.0 * n
                    out.append(n)
                    kc += n
                    if any(it[1] <= t for it in cs[kc:kc + 200]):
                        return None
                return out
            rate, sched = next((r, o) for r, o in ((r, plan(r)) for r in range(180, 320)) if o is not None)
            if DEBUG:
                print("rate", rate)
            if DEBUG:
                print(''.join('x' if t in xat else str(o) for t, o in enumerate(sched)))

            for t, (kind, p, idx) in enumerate(seq):
                if kind == 'b' and idx == 0 and p % 2 == 0:
                    if p == 0:
                        xraw(0)
                    if p // 2 + 1 < nq:
                        xraw(p // 2 + 1)
                if kind == 'A':
                    res = [leaf_job(*jb) for jb in ap[p]][-ANC]
                else:
                    res = run(kind, p, idx)
                if t in xat:
                    xmega(*xat[t], anchors(res[0:RC - XEARLY], 4))
                n = sched[t]
                if n:
                    an = anchors(res, n)
                    for k in range(n):
                        c16(*cs.pop(0)[2], an[k])
                if kind == 'm':
                    if p == ns - 1:
                        if idx == 3:
                            out_dma(p, pl.ds(0, 256))
                        elif idx == 6:
                            out_dma(p, pl.ds(256, 256))
                    elif idx == 6:
                        out_dma(p, slice(None))
            assert not cs
            n = 2 * ns * RC
            for c in range(NC):
                h_ref[c, 0:16, :] = h_ref[c, n:n + 16, :]

        @pl.when(j == 0)
        def _():
            for g in range(5):
                start_group(g)
            xbuf[R:R + 16, :] = jnp.zeros((16, D), bf16)
            for c in range(NC):
                h_ref[c, 0:8, :] = jnp.zeros((8, 128), f32)

            todo = []

            def attach(res, n):
                n = min(n, len(todo))
                if n:
                    an = anchors(res, 2 * n)
                    for k in range(n):
                        cpair(*todo.pop(0), an[2 * k:2 * k + 2])

            def pw1_rows(c, lo=0, hi=X0, raw=True):
                xq = xbuf[lo:hi, :]
                a = jnp.dot(xq, w1tile(c, raw), preferred_element_type=f32)
                attach(a, 3 * P0)
                b = jnp.dot(xq, w1tile(NC + c, raw), preferred_element_type=f32)
                attach(b[0:hi - lo - 80], 2 * P0)
                g = a * (1.0 + jnp.tanh(0.5 * b))
                n = min(hi, X0 - 8) - lo
                h_ref[c, 8 + lo:8 + lo + n, :] = g[0:n]
                if hi == X0:
                    todo.extend((p, c // 2, i, c % 2) for p in range(P0) for i in IORD)

            wait_group(0)
            pw1_rows(0, 0, XA)
            wait_group(1)
            pw1_rows(0, XA, X0, raw=False)
            dwf = dwraw[...].astype(f32) * 0.25
            for c in range(NC):
                for k in range(K):
                    dwb[c * K + k] = jnp.broadcast_to(dwf[k:k + 1, c * 128:(c + 1) * 128], (8, 128))
            wait_group(2)
            if XST == 2:
                xb_copy(0).start()
            pw1_rows(1)
            wait_group(3)
            if XST == 3:
                xb_copy(0).start()
            pw1_rows(2)
            pw1_rows(3)
            wait_group(4)

            ctx.direct = (P0, P0 + 1)
            pipeline([(s[0], int(s[1:])) for s in PSEQ.split('.')], P0, QP // 2, todo, True, False)
            pltpu.make_async_copy(obuf.at[pl.ds(0, TP), :], o_hbm.at[pl.ds(0, TP), :], sem_out).start()

        @pl.when(j > 0)
        def _():
            i = j - 1
            xb_copy(i).wait()

            @pl.when(j < NB)
            def _():
                xb_copy(j).start()

            base = pl.multiple_of(TP + i * TB, 16)
            masks = {}
            last_flag = i == NB - 1
            if bnd_q == 0:
                last_flag = jnp.logical_or(last_flag, i == bnd_it - 1)
            else:
                masks[bnd_q * RC - 16] = ('last', i == bnd_it)
            masks[TB - 16] = ('last', last_flag)
            masks[bnd_q * RC] = ('first', i == bnd_it)
            ctx.xv, ctx.ov = xbuf.at[pl.ds(base, TB + 16), :], obuf.at[pl.ds(base, TB), :]
            ctx.obase, ctx.masks, ctx.direct = base, masks, (0,)
            ctx.direct, ctx.xrr = (0, 1), XRR
            pipeline2(QB // 4)

        @pl.when(j == NB)
        def _():
            pltpu.make_async_copy(o_hbm, o_hbm, sem_out).wait()

    opts = dict(dimension_semantics=("arbitrary",), vmem_limit_bytes=100 * 1024 * 1024)
    for name in ("disable_bounds_checks", "disable_semaphore_checks"):
        if hasattr(pltpu.CompilerParams, name):
            opts[name] = True

    out = pl.pallas_call(
        kernel,
        grid=(NB + 1,),
        in_specs=[pl.BlockSpec(memory_space=pl.ANY)] * 4,
        out_specs=pl.BlockSpec(memory_space=pl.ANY),
        out_shape=jax.ShapeDtypeStruct((R, D), x.dtype),
        scratch_shapes=[
            pltpu.VMEM((R + 16, D), bf16),
            pltpu.VMEM((2 * NC, D, 128), bf16),
            pltpu.VMEM((NC, D, 128), bf16),
            pltpu.VMEM((K, D), bf16),
            pltpu.VMEM((D // 2, 2 * D), u32),
            pltpu.VMEM((NC * K, 8, 128), f32),
            pltpu.VMEM((NC, HR, 128), f32),
            pltpu.VMEM((R, D), bf16),
            pltpu.VMEM((7 * 128, 256), u32),
            pltpu.VMEM((7 * 128, 256), u32),
            pltpu.VMEM((2, RING * 5 * RH, 256), u32),
            pltpu.VMEM((2, RING * 2 * RH, D), u32),
            pltpu.VMEM((2, RING * 7 * RH, 256), u32),
            pltpu.VMEM((2, 4 * RC, D), f32),
            pltpu.VMEM((25 * 64, 256), u32),
            pltpu.VMEM((2, QRING * 25 * RH, 256), u32),
            pltpu.VMEM((2, 32 * RC, 128), f32),
            pltpu.SemaphoreType.DMA((5,)),
            pltpu.SemaphoreType.DMA,
            pltpu.SemaphoreType.DMA,
        ],
        compiler_params=pltpu.CompilerParams(**opts),
    )(x.reshape(R, D), w_pw1, dw, w_pw2)
    return out.reshape(B, T, D)
```

```python
import jax
import jax.numpy as jnp
import jax.experimental.pallas as pl
import jax.experimental.pallas.tpu as pltpu

RC = 80
NP = 6
XA = 176
QP = 12
QB = 44
PSEQ = 'b3.b4.a3.a4.b5.a5.m0.m1.m2.m3.m4.m5'
LAGQ = 1
RESV = 35
SDL = 2
SLAG = 2
XDL = 2
XU0 = 7
XU = 5
RING = 12
QRING = 3
XRR = 8
XPOS = (1, 4, 7, 10, 13)
BORD = (0, 1, 2, 3, 1, 0, 3, 2)
IORD = (0, 2, 4, 1, 3)
T12 = ((0, 2), (1, 3))
SA = ((1, 0, 0, 1), (0, 0, 1, 1), (1, 0, 0, 0), (0, 0, 0, 1), (1, 1, 0, 0), (-1, 0, 1, 0), (0, 1, 0, -1))
SB = ((1, 0, 0, 1), (1, 0, 0, 0), (0, 1, 0, -1), (-1, 0, 1, 0), (0, 0, 0, 1), (1, 1, 0, 0), (0, 0, 1, 1))
MORD = (1, 3, 2, 4, 0, 6, 5)


@jax.jit
def pallas_standalone__conformer_conv_module__speech_kernel(x, w_pw1, dw, w_pw2):
    B, T, D = x.shape
    K = dw.shape[0]
    pad = K // 2
    R = B * T
    NC = D // 128
    P0 = NP // 2
    assert T % RC == 0 and pad <= 8 and NC == 4 and NP % 2 == 0 and QB % 4 == 0
    f32, bf16, u32 = jnp.float32, jnp.bfloat16, jnp.uint32
    NPAIR = RC // 16
    RH = RC // 2
    X0 = NP * RC + 16
    TP = QP * RC
    TB = QB * RC
    NB = (R - TP) // TB
    assert TP + NB * TB == R and B == 2 and TP < T
    gq = (T - TP) // RC
    bnd_it, bnd_q = gq // QB, gq % QB
    HR = max(TP, TB) + 16
    X1 = TP + 8 * NB
    XN = TB - 8

    def kernel(x_hbm, w1_hbm, dw_hbm, w2_hbm, o_hbm,
               xbuf, w1raw, w2raw, dwraw, w1p, dwb, h_ref, obuf,
               wsa, wsm, xs_all, xr_all, ss_all, g_all, wsa2, x2_all, t_all, sem_in, sem_x, sem_out):
        j = pl.program_id(0)
        sub8 = jax.lax.broadcasted_iota(jnp.int32, (8, 128), 0)
        never = sub8 > j + 1000
        xs_ref, xr_ref, ss_ref, g_ref = xs_all.at[j % 2], xr_all.at[j % 2], ss_all.at[j % 2], g_all.at[j % 2]

        def pin(v, dep):
            if dep is None:
                return v
            if v.shape[0] == 8:
                return jnp.where(never, dep, v)
            return jnp.concatenate([jnp.where(never, dep, v[0:8]), v[8:]], axis=0)

        def st_packed(ref, r, t, v):
            ref[r:r + 8, t * 128:(t + 1) * 128] = pltpu.bitcast(v.astype(bf16), u32)

        def w1_copy(col, s):
            return pltpu.make_async_copy(w1_hbm.at[:, pl.ds(col * 128, 128)], w1raw.at[col], sem_in.at[s])

        def w2_copy(col, s):
            return pltpu.make_async_copy(w2_hbm.at[:, pl.ds(col * 128, 128)], w2raw.at[col], sem_in.at[s])

        def x_copy(lo, hi, s):
            return pltpu.make_async_copy(x_hbm.at[pl.ds(lo, hi - lo), :], xbuf.at[pl.ds(lo, hi - lo), :], sem_in.at[s])

        groups = [
            [x_copy(0, XA, 0), w1_copy(0, 0), w1_copy(NC, 0)],
            [x_copy(XA, X0, 1), pltpu.make_async_copy(dw_hbm, dwraw, sem_in.at[1])],
            [w1_copy(1, 2), w1_copy(NC + 1, 2)],
            [w1_copy(2, 3), w1_copy(NC + 2, 3), w1_copy(3, 3), w1_copy(NC + 3, 3)],
            [x_copy(X0, X1, 4)] + [w2_copy(n, 4) for n in range(NC)],
        ]

        def xb_copy(i):
            lo = X1 + i * XN
            if not isinstance(lo, int):
                lo = pl.multiple_of(lo, 8)
            return pltpu.make_async_copy(x_hbm.at[pl.ds(lo, XN), :], xbuf.at[pl.ds(lo, XN), :], sem_x)

        class ctx:
            xv, ov, obase, masks, direct, xrr = xbuf, obuf, 0, {}, (), 2 * RING

        def start_group(g):
            for cp in groups[g]:
                cp.start()

        def wait_group(g):
            for cp in groups[g]:
                cp.wait()

        def w1tile(col, raw=False):
            if raw:
                wt = w1raw[col]
                w1p[:, col * 128:(col + 1) * 128] = pltpu.bitcast(wt, u32)
                return wt
            return pltpu.bitcast(w1p[:, col * 128:(col + 1) * 128], bf16)

        sub16 = jax.lax.broadcasted_iota(jnp.int32, (16, 128), 0)

        def conv16(c, o, dep, ws):
            mode, flag = ctx.masks.get(o, (None, None))
            acc = None
            for k in range(K):
                v = h_ref[c, pl.ds(8 + o + k - pad, 16), :]
                if mode == 'last' and k > pad:
                    v = jnp.where(sub16 < jnp.where(flag, 16 + pad - k, 16), v, 0.0)
                elif mode == 'first' and k < pad:
                    v = jnp.where(sub16 >= jnp.where(flag, pad - k, 0), v, 0.0)
                w = jnp.concatenate([pin(ws[k], dep) if k == K - 1 else ws[k]] * 2, axis=0)
                t = v * w
                acc = t if acc is None else acc + t
            return acc + acc * jnp.tanh(acc)

        sv = {}

        def cpair(p, l, i, half, deps):
            for u in range(2):
                c16(p, l, i, half, u, deps[u])

        def c16(p, l, i, half, u, dep):
            c = T12[half][l]
            y = conv16(c, (2 * p + u) * RC + 16 * i, dep, [dwb[c * K + k] for k in range(K)])

            def put(n, v):
                st_packed(ss_ref, ((p % RING) * 7 + n) * RH + 8 * i, l, v)
            s = sv.setdefault((p, l, i), {})
            s[(u, half)] = y
            if (u, half) == (0, 0):
                put(2, y)
            elif (u, half) == (1, 0):
                put(5, y - s[(0, 0)])
            elif (u, half) == (0, 1):
                put(4, s[(0, 0)] + y)
            else:
                put(0, s[(0, 0)] + y)
                put(1, s[(1, 0)] + y)
                put(3, y)
                put(6, s[(0, 1)] - y)
                del sv[(p, l, i)]

        def xprep(p, i, l, dep):
            def ld(q, t):
                r = q * RC + 8 + 16 * i
                cs = slice(t * 128, (t + 1) * 128)
                return jnp.concatenate([ctx.xv[r:r + 8, cs].astype(f32), ctx.xv[r + 8:r + 16, cs].astype(f32)], axis=0)
            q1, q2 = 2 * p, 2 * p + 1
            a11, a12, a21, a22 = pin(ld(q1, l), dep), ld(q1, l + 2), ld(q2, l), pin(ld(q2, l + 2), dep)
            for n, v in enumerate([a11 + a22, a21 + a22, a11 + a12, a21 - a11, a12 - a22]):
                st_packed(xs_ref, ((p % RING) * 5 + n) * RH + 8 * i, l, v)
            for u, t, v in [(0, l, a11), (0, l + 2, a12), (1, l, a21), (1, l + 2, a22)]:
                st_packed(xr_ref, ((p % RING) * 2 + u) * RH + 8 * i, t, v)

        def wprep(which, l, kl, i, dep):
            if which == 'a':
                raw, dst, kt, nt = w1raw, wsa, ((0, 1), (2, 3)), T12
            else:
                raw, dst, kt, nt = w2raw, wsm, T12, ((0, 2), (1, 3))

            def ld(kh, nh):
                r = kt[kh][kl] * 128 + 16 * i
                return raw[nt[nh][l], r:r + 16, :].astype(f32)
            b11, b12, b21, b22 = pin(ld(0, 0), dep), ld(0, 1), ld(1, 0), pin(ld(1, 1), dep)
            for n, v in enumerate([b11 + b22, b11, b12 - b22, b21 - b11, b22, b11 + b12, b21 + b22]):
                st_packed(dst, n * 128 + kl * 64 + 8 * i, l, v)

        def comb(coef, vals):
            pos_ = [v for s, v in zip(coef, vals) if s > 0]
            neg_ = [v for s, v in zip(coef, vals) if s < 0]
            acc = pos_[0]
            for v in pos_[1:]:
                acc = acc + v
            for v in neg_:
                acc = acc - v
            return acc

        def leaves(S, X, deps, emit):
            if deps is not None:
                for k, (o, n) in enumerate(((3, 3), (3, 0), (0, 3), (0, 0))):
                    X[o][n] = pin(X[o][n], deps[k])
            for I in (3, 1, 6, 2, 0, 4, 5):
                O = [comb(S[I], [X[o][n] for o in range(4)]) for n in range(4)]
                for J in (3, 1, 6, 2, 0, 4, 5):
                    emit(I, J, comb(S[J], O))

        x2_ref, t_ref = x2_all.at[j % 2], t_all.at[j % 2]

        def xmega(Q, i, deps):
            def ld(o, n):
                q = 4 * Q + 2 * (o // 2) + n // 2
                t = 2 * (o % 2) + n % 2
                r = q * RC + 8 + 16 * i
                cs = slice(t * 128, (t + 1) * 128)
                return jnp.concatenate([ctx.xv[r:r + 8, cs].astype(f32), ctx.xv[r + 8:r + 16, cs].astype(f32)], axis=0)
            X = [[ld(o, n) for n in range(4)] for o in range(4)]

            def emit(I, J, v):
                if not (I in (2, 3) and J in (2, 3)):
                    st_packed(x2_ref, ((Q % QRING) * 25 + (7 * I + J) // 2) * RH + 8 * i, (7 * I + J) % 2, v)
            leaves(SA, X, deps, emit)

        def xraw(Q):
            for q in range(4 * Q, 4 * Q + 4):
                r = (q % XRR) * RH
                xr_ref[r:r + RH, :] = pltpu.bitcast(ctx.xv[q * RC + 8:(q + 1) * RC + 8, :], u32)

        def wmega(i, deps):
            def ld(o, n):
                r = (2 * (o // 2) + n // 2) * 128 + 16 * i
                return w1raw[2 * (o % 2) + n % 2, r:r + 16, :].astype(f32)
            X = [[ld(o, n) for n in range(4)] for o in range(4)]
            leaves(SB, X, deps, lambda I, J, v: st_packed(wsa2, (7 * I + J) // 2 * 64 + 8 * i, (7 * I + J) % 2, v))

        slot = [0]
        inner, outer = {}, {}

        def keep(name, v):
            slot[0] = (slot[0] + 1) % 32
            t_ref[slot[0] * RC:(slot[0] + 1) * RC, :] = v
            outer[name] = slot[0]

        def get(name):
            s = outer[name]
            return t_ref[s * RC:(s + 1) * RC, :]

        def fin2(Q, o, n, v):
            q = 4 * Q + 2 * (o // 2) + n // 2
            c = 2 * (o % 2) + n % 2
            g = g_ref[(q % 4) * RC:(q % 4 + 1) * RC, c * 128:(c + 1) * 128]
            h_ref[c, 16 + q * RC:16 + (q + 1) * RC, :] = v * g

        def outer_step(Q, I, n, m):
            if I == 1:
                keep(('m2', n), m)
            elif I == 3:
                fin2(Q, 2, n, get(('m2', n)) + m)
                keep(('t11', n), m)
            elif I == 2:
                keep(('m3', n), m)
                keep(('t22', n), m - get(('m2', n)))
            elif I == 4:
                fin2(Q, 1, n, get(('m3', n)) + m)
                keep(('t11', n), get(('t11', n)) - m)
            elif I == 0:
                keep(('t11', n), get(('t11', n)) + m)
                keep(('t22', n), get(('t22', n)) + m)
            elif I == 6:
                fin2(Q, 0, n, get(('t11', n)) + m)
            else:
                fin2(Q, 3, n, get(('t22', n)) + m)

        def leaf_job(Q, I, J):
            e = 7 * I + J
            if I in (2, 3) and J in (2, 3):
                o, n = 3 * (I - 2), 3 * (J - 2)
                q = 4 * Q + 2 * (o // 2) + n // 2
                t = 2 * (o % 2) + n % 2
                r = (q % XRR) * RH
                a = xr_ref[r:r + RH, t * 128:(t + 1) * 128]
            else:
                r = ((Q % QRING) * 25 + e // 2) * RH
                a = x2_ref[r:r + RH, (e % 2) * 128:(e % 2 + 1) * 128]
            w = wsa2[e // 2 * 64:(e // 2 + 1) * 64, (e % 2) * 128:(e % 2 + 1) * 128]
            m = jnp.dot(pltpu.bitcast(a, bf16), pltpu.bitcast(w, bf16), preferred_element_type=f32)
            s = inner
            if J == 1:
                s['m2'] = m
            elif J == 3:
                outer_step(Q, I, 2, s['m2'] + m)
                s['t11'] = m
            elif J == 2:
                s['m3'] = m
                s['t22'] = m - s.pop('m2')
            elif J == 4:
                outer_step(Q, I, 1, s.pop('m3') + m)
                s['t11'] = s['t11'] - m
            elif J == 0:
                s['t11'] = s['t11'] + m
                s['t22'] = s['t22'] + m
            elif J == 6:
                outer_step(Q, I, 0, s.pop('t11') + m)
            else:
                outer_step(Q, I, 3, s.pop('t22') + m)
            return m

        def lhs(kind, p, n):
            pr = p % RING
            if kind == 'm':
                v = ss_ref[(pr * 7 + n) * RH:(pr * 7 + n + 1) * RH, :]
            elif n == 2:
                v = xr_ref[2 * pr * RH:(2 * pr + 1) * RH, 0:256]
            elif n == 3:
                v = xr_ref[(2 * pr + 1) * RH:(2 * pr + 2) * RH, 256:512]
            else:
                m = {0: 0, 1: 1, 4: 2, 5: 3, 6: 4}[n]
                v = xs_ref[(pr * 5 + m) * RH:(pr * 5 + m + 1) * RH, :]
            return pltpu.bitcast(v, bf16)

        def prod(kind, p, n, l):
            w = wsa if kind == 'a' else wsm
            wt = w[n * 128:(n + 1) * 128, :] if l is None else w[n * 128:(n + 1) * 128, l * 128:(l + 1) * 128]
            return jnp.dot(lhs(kind, p, n), pltpu.bitcast(wt, bf16), preferred_element_type=f32)

        def fin(kind, p, l, rh, ch, v):
            q = 2 * p + rh
            if kind == 'a':
                c = T12[ch][l]
                g = g_ref[(q % 4) * RC:(q % 4 + 1) * RC, c * 128:(c + 1) * 128]
                h_ref[c, 16 + q * RC:16 + (q + 1) * RC, :] = v * g
            else:
                c = 2 * l + ch
                ctx.ov[q * RC:(q + 1) * RC, c * 128:(c + 1) * 128] = v.astype(bf16)

        st = {}

        bres = {}

        def run(kind, p, idx):
            if kind == 'b' and ctx.xrr == XRR and p not in ctx.direct:
                k = 8 * (p % 2) + idx
                if k % 4 == 0:
                    r, c = (2 * (p - p % 2) % XRR) * RH, k // 4
                    xq = pltpu.bitcast(xr_ref[r:r + 4 * RH, :], bf16)
                    b = jnp.dot(xq, w1tile(NC + c), preferred_element_type=f32)
                    g_ref[:, c * 128:(c + 1) * 128] = 1.0 + jnp.tanh(0.5 * b)
                    bres[0] = b
                return bres[0][(k % 4) * RC:(k % 4 + 1) * RC]
            if kind == 'b':
                u, c = idx % 2, BORD[idx]
                q = 2 * p + u
                if p in ctx.direct:
                    xq = ctx.xv[q * RC + 8:(q + 1) * RC + 8, :]
                else:
                    r = (q % ctx.xrr) * RH
                    xq = pltpu.bitcast(xr_ref[r:r + RH, :], bf16)
                b = jnp.dot(xq, w1tile(NC + c), preferred_element_type=f32)
                g_ref[(q % 4) * RC:(q % 4 + 1) * RC, c * 128:(c + 1) * 128] = 1.0 + jnp.tanh(0.5 * b)
                return b
            l = 0 if idx < 3 else 1
            step = idx if idx < 3 else idx - 4
            if idx == 3:
                m6 = prod(kind, p, 5, None)
                fin(kind, p, 0, 1, 1, st.pop('t22') + m6[:, 0:128])
                st['t22'] = m6[:, 128:256]
                return m6[:, 128:256]
            if step == 0:
                m2, m4 = prod(kind, p, 1, l), prod(kind, p, 3, l)
                fin(kind, p, l, 1, 0, m2 + m4)
                st['t11'] = m4
                st['t22'] = m2 if l == 0 else st['t22'] - m2
                return m4
            if step == 1:
                m3, m5 = prod(kind, p, 2, l), prod(kind, p, 4, l)
                fin(kind, p, l, 0, 1, m3 + m5)
                st['t11'] = st['t11'] - m5
                st['t22'] = m3 - st['t22'] if l == 0 else st['t22'] + m3
                return m5
            m1, m7 = prod(kind, p, 0, l), prod(kind, p, 6, l)
            fin(kind, p, l, 0, 0, st.pop('t11') + m1 + m7)
            if l == 0:
                st['t22'] = st['t22'] + m1
            else:
                fin(kind, p, l, 1, 1, st.pop('t22') + m1)
            return m7

        def out_dma(p, cols):
            dst = ctx.obase + 2 * p * RC
            if not isinstance(dst, int):
                dst = pl.multiple_of(dst, 16)
            pltpu.make_async_copy(ctx.ov.at[pl.ds(2 * p * RC, 2 * RC), cols],
                                  o_hbm.at[pl.ds(dst, 2 * RC), cols], sem_out).start()

        def anchors(res, n):
            nv = res.shape[0] // 8
            ks = [((2 * k + 1) * nv) // (2 * n) for k in range(n)]
            return [res[8 * k:8 * k + 8] for k in ks]

        def pipeline(groups_, p0, ns, todo):
            seq = [(kind, p, i) for kind, p in groups_ for i in range(8 if kind == 'b' else 7)]
            pos = {it: t for t, it in enumerate(seq)}
            sm, cs = [], []
            for w, dl in (('a', pos[('a', p0, 0)]), ('m', pos[('m', 0, 0)])):
                sm += [(0, dl - XDL, wprep, (w, l, kl, i)) for l in range(2) for kl in range(2) for i in range(8)]
            for p in range(p0, ns):
                dl = pos[('a' if p in ctx.direct else 'b', p, 0)] - XDL
                av = pos[('a', p - RING, 6)] + 1 if p - RING >= p0 else 0
                sm += [(av, dl, xprep, (p, i, l)) for i in range(NPAIR) for l in range(2)]
            sm.sort(key=lambda it: it[1])
            cs += [(0, pos[('m', it[0], 0)] - SDL, it) for it in todo]
            for p in range(p0, ns):
                for l in range(2):
                    for i in IORD:
                        for half in range(2):
                            av = pos[('a', p, (2 + half) if l == 0 else 6)] + SLAG
                            cs.append((av, pos[('m', p, 0)] - SDL, (p, l, i, half)))

            def plan(rate):
                out, kc, ks, credit, worst = [], 0, 0, 0.0, 0
                for t in range(len(seq)):
                    c_slack = min([it[1] - t - i for i, it in enumerate(cs[kc:kc + 80])], default=99)
                    s_slack = min([it[1] - t - i // XU for i, it in enumerate(sm[ks:ks + 80])], default=99)
                    nc = len([it for it in cs[kc:kc + (2 if c_slack < 0 else 1)] if it[0] <= t])
                    if s_slack <= 0 and c_slack > 0:
                        nc = 0
                    if nc == 0 or s_slack <= 0:
                        nx = XU0 if (t < 15 and nc == 0) else XU
                    else:
                        credit = min(credit + rate, 1.5)
                        nx = 1 if credit >= 1.0 else 0
                    nx = len([it for it in sm[ks:ks + nx] if it[0] <= t])
                    if nc:
                        credit -= min(nx, 1)
                    worst += (nc > 1) + (nc > 0 and nx > 1)
                    out.append((nc, nx))
                    kc += nc
                    ks += nx
                    assert (kc == len(cs) or cs[kc][1] > t) and (ks == len(sm) or sm[ks][1] > t)
                return worst, out
            plans = [plan(r / 100.0) for r in range(0, 101, 2)]
            best = min(w for w, o in plans)
            sched = next(o for w, o in plans if w == best)

            for t, (kind, p, idx) in enumerate(seq):
                res = run(kind, p, idx)
                nc, nx = sched[t]
                if len(seq) - 9 <= t < len(seq) - 1:
                    wmega(t - (len(seq) - 9), anchors(res, 4))
                if nc + nx:
                    an = anchors(res, 2 * nc + nx)
                    for k in range(nx):
                        it = sm.pop(0)
                        it[2](*it[3], an[k])
                    for k in range(nc):
                        cpair(*cs.pop(0)[2], an[nx + 2 * k:nx + 2 * k + 2])
            assert not sm and not cs
            n = 2 * ns * RC
            for c in range(NC):
                h_ref[c, 0:16, :] = h_ref[c, n:n + 16, :]

        def pipeline2(nq):
            jobs = [(Q, I, J) for Q in range(nq) for I in MORD for J in MORD]
            ap = [jobs[k:k + 4] for k in range(0, len(jobs), 4)]
            ns = 2 * nq
            seq, mdone = [], 0
            for Q in range(nq):
                seq += [('b', 2 * Q + k // 8, k % 8) for k in range(16)]
                seq += [('A', k, 0) for k in range(len(ap)) if ap[k][0][0] == Q]
                for p in (2 * (Q - LAGQ), 2 * (Q - LAGQ) + 1):
                    if p >= 0 and 7 * (ns - 1 - p) > RESV:
                        seq += [('m', p, i) for i in range(7)]
                        mdone = p + 1
            seq += [('m', p, i) for p in range(mdone, ns) for i in range(7)]
            pos = {it: t for t, it in enumerate(seq)}
            jpos = {jb: pos[('A', k, 0)] for k, js in enumerate(ap) for jb in js}
            lastp = {2: 3, 1: 4, 0: 6, 3: 5}
            tfin = {}
            for Q in range(nq):
                for o in range(4):
                    for n in range(4):
                        tfin[(4 * Q + 2 * (o // 2) + n // 2, 2 * (o % 2) + n % 2)] = jpos[(Q, lastp[o], lastp[n])]
            quads = []
            for p in range(ns):
                for l in range(2):
                    for i in IORD:
                        qs = [2 * p, 2 * p + 1] + ([2 * p - 1] if i == 0 and p > 0 else [])
                        av = max(tfin[(q, 2 * l + h)] for q in qs for h in range(2)) + SLAG
                        quads.append((av, pos[('m', p, 0)] - SDL, p, l, i))
            quads.sort(key=lambda it: it[0])
            cs = [(av, dl, (p, l, i, half, u)) for av, dl, p, l, i in quads for half in range(2) for u in range(2)]
            xat = {}
            free = [t for t in range(16) if t % 4 != 3]
            for Q in range(nq):
                for i in range(NPAIR):
                    if free and Q < QRING:
                        t = free.pop(0)
                    else:
                        t = pos[('b', 2 * (Q - 1), 0)] + XPOS[i]
                    assert t <= jpos[(Q, MORD[0], MORD[0])] - XDL and t not in xat
                    assert Q < QRING or t > jpos[(Q - QRING, MORD[6], MORD[6])]
                    xat[t] = (Q, i)

            icost = (20, 0, 10, 10, 20, 10, 10)
            ocost = (20, 0, 10, 20, 30, 20, 20)
            own = []
            for t, (kind, p, idx) in enumerate(seq):
                if kind == 'b':
                    v = 60
                elif kind == 'm':
                    v = (40, 60, 60, 40, 50, 60, 70)[idx]
                else:
                    v = sum(icost[J] + (ocost[I] if J in (3, 4, 5, 6) else 0) for _, I, J in ap[p])
                own.append(v + (191 if t in xat else 0))

            def plan(rate):
                out, kc, credit = [], 0, 0.0
                for t in range(len(seq)):
                    credit = min(credit, 35.0) + rate - own[t]
                    n = max(0, min(3, int(credit / 69.0 + 0.5)))
                    n = next((k for k, it in enumerate(cs[kc:kc + n]) if it[0] > t), min(n, len(cs) - kc))
                    credit -= 69.0 * n
                    out.append(n)
                    kc += n
                    if any(it[1] <= t for it in cs[kc:kc + 200]):
                        return None
                return out
            rate, sched = next((r, o) for r, o in ((r, plan(r)) for r in range(180, 320)) if o is not None)

            for t, (kind, p, idx) in enumerate(seq):
                if kind == 'b' and idx == 0 and p % 2 == 0:
                    if p == 0:
                        xraw(0)
                    if p // 2 + 1 < nq:
                        xraw(p // 2 + 1)
                if kind == 'A':
                    res = [leaf_job(*jb) for jb in ap[p]][-1]
                else:
                    res = run(kind, p, idx)
                if t in xat:
                    xmega(*xat[t], anchors(res, 4))
                n = sched[t]
                if n:
                    an = anchors(res, n)
                    for k in range(n):
                        c16(*cs.pop(0)[2], an[k])
                if kind == 'm':
                    if p == ns - 1:
                        if idx == 3:
                            out_dma(p, pl.ds(0, 256))
                        elif idx == 6:
                            out_dma(p, pl.ds(256, 256))
                    elif idx == 6:
                        out_dma(p, slice(None))
            assert not cs
            n = 2 * ns * RC
            for c in range(NC):
                h_ref[c, 0:16, :] = h_ref[c, n:n + 16, :]

        @pl.when(j == 0)
        def _():
            for g in range(5):
                start_group(g)
            xbuf[R:R + 16, :] = jnp.zeros((16, D), bf16)
            for c in range(NC):
                h_ref[c, 0:8, :] = jnp.zeros((8, 128), f32)

            todo = []

            def attach(res, n):
                n = min(n, len(todo))
                if n:
                    an = anchors(res, 2 * n)
                    for k in range(n):
                        cpair(*todo.pop(0), an[2 * k:2 * k + 2])

            def pw1_rows(c, lo=0, hi=X0, raw=True):
                xq = xbuf[lo:hi, :]
                a = jnp.dot(xq, w1tile(c, raw), preferred_element_type=f32)
                attach(a, 3 * P0)
                b = jnp.dot(xq, w1tile(NC + c, raw), preferred_element_type=f32)
                attach(b[0:hi - lo - 80], 2 * P0)
                g = a * (1.0 + jnp.tanh(0.5 * b))
                n = min(hi, X0 - 8) - lo
                h_ref[c, 8 + lo:8 + lo + n, :] = g[0:n]
                if hi == X0:
                    todo.extend((p, c // 2, i, c % 2) for p in range(P0) for i in IORD)

            wait_group(0)
            pw1_rows(0, 0, XA)
            wait_group(1)
            pw1_rows(0, XA, X0, raw=False)
            dwf = dwraw[...].astype(f32) * 0.25
            for c in range(NC):
                for k in range(K):
                    dwb[c * K + k] = jnp.broadcast_to(dwf[k:k + 1, c * 128:(c + 1) * 128], (8, 128))
            wait_group(2)
            xb_copy(0).start()
            pw1_rows(1)
            wait_group(3)
            pw1_rows(2)
            pw1_rows(3)
            wait_group(4)

            ctx.direct = (P0, P0 + 1)
            pipeline([(s[0], int(s[1:])) for s in PSEQ.split('.')], P0, QP // 2, todo)
            pltpu.make_async_copy(obuf.at[pl.ds(0, TP), :], o_hbm.at[pl.ds(0, TP), :], sem_out).start()

        @pl.when(j > 0)
        def _():
            i = j - 1
            xb_copy(i).wait()

            @pl.when(j < NB)
            def _():
                xb_copy(j).start()

            base = pl.multiple_of(TP + i * TB, 16)
            masks = {}
            last_flag = i == NB - 1
            if bnd_q == 0:
                last_flag = jnp.logical_or(last_flag, i == bnd_it - 1)
            else:
                masks[bnd_q * RC - 16] = ('last', i == bnd_it)
            masks[TB - 16] = ('last', last_flag)
            masks[bnd_q * RC] = ('first', i == bnd_it)
            ctx.xv, ctx.ov = xbuf.at[pl.ds(base, TB + 16), :], obuf.at[pl.ds(base, TB), :]
            ctx.obase, ctx.masks, ctx.direct = base, masks, (0,)
            ctx.direct, ctx.xrr = (0, 1), XRR
            pipeline2(QB // 4)

        @pl.when(j == NB)
        def _():
            pltpu.make_async_copy(o_hbm, o_hbm, sem_out).wait()

    opts = dict(dimension_semantics=("arbitrary",), vmem_limit_bytes=100 * 1024 * 1024)
    for name in ("disable_bounds_checks", "disable_semaphore_checks"):
        if hasattr(pltpu.CompilerParams, name):
            opts[name] = True

    out = pl.pallas_call(
        kernel,
        grid=(NB + 1,),
        in_specs=[pl.BlockSpec(memory_space=pl.ANY)] * 4,
        out_specs=pl.BlockSpec(memory_space=pl.ANY),
        out_shape=jax.ShapeDtypeStruct((R, D), x.dtype),
        scratch_shapes=[
            pltpu.VMEM((R + 16, D), bf16),
            pltpu.VMEM((2 * NC, D, 128), bf16),
            pltpu.VMEM((NC, D, 128), bf16),
            pltpu.VMEM((K, D), bf16),
            pltpu.VMEM((D // 2, 2 * D), u32),
            pltpu.VMEM((NC * K, 8, 128), f32),
            pltpu.VMEM((NC, HR, 128), f32),
            pltpu.VMEM((R, D), bf16),
            pltpu.VMEM((7 * 128, 256), u32),
            pltpu.VMEM((7 * 128, 256), u32),
            pltpu.VMEM((2, RING * 5 * RH, 256), u32),
            pltpu.VMEM((2, RING * 2 * RH, D), u32),
            pltpu.VMEM((2, RING * 7 * RH, 256), u32),
            pltpu.VMEM((2, 4 * RC, D), f32),
            pltpu.VMEM((25 * 64, 256), u32),
            pltpu.VMEM((2, QRING * 25 * RH, 256), u32),
            pltpu.VMEM((2, 32 * RC, 128), f32),
            pltpu.SemaphoreType.DMA((5,)),
            pltpu.SemaphoreType.DMA,
            pltpu.SemaphoreType.DMA,
        ],
        compiler_params=pltpu.CompilerParams(**opts),
    )(x.reshape(R, D), w_pw1, dw, w_pw2)
    return out.reshape(B, T, D)
```

```python
import jax
import jax.numpy as jnp
import jax.experimental.pallas as pl
import jax.experimental.pallas.tpu as pltpu

RC = 80
NP = 6
XA = 176
QP = 12
QB = 44
PSEQ = 'b3.b4.a3.a4.b5.a5.m0.m1.m2.m3.m4.m5'
LAGQ = 1
RESV = 35
SDL = 2
SLAG = 2
XDL = 2
XU0 = 7
XU = 5
RING = 12
QRING = 3
XRR = 8
XPOS = (1, 4, 7, 10, 13)
BORD = (0, 1, 2, 3, 1, 0, 3, 2)
IORD = (0, 2, 4, 1, 3)
T12 = ((0, 2), (1, 3))
SA = ((1, 0, 0, 1), (0, 0, 1, 1), (1, 0, 0, 0), (0, 0, 0, 1), (1, 1, 0, 0), (-1, 0, 1, 0), (0, 1, 0, -1))
SB = ((1, 0, 0, 1), (1, 0, 0, 0), (0, 1, 0, -1), (-1, 0, 1, 0), (0, 0, 0, 1), (1, 1, 0, 0), (0, 0, 1, 1))
MORD = (1, 3, 2, 4, 0, 6, 5)


@jax.jit
def pallas_standalone__conformer_conv_module__speech_kernel(x, w_pw1, dw, w_pw2):
    B, T, D = x.shape
    K = dw.shape[0]
    pad = K // 2
    R = B * T
    NC = D // 128
    P0 = NP // 2
    assert T % RC == 0 and pad <= 8 and NC == 4 and NP % 2 == 0 and QB % 4 == 0
    f32, bf16, u32 = jnp.float32, jnp.bfloat16, jnp.uint32
    NPAIR = RC // 16
    RH = RC // 2
    X0 = NP * RC + 16
    TP = QP * RC
    TB = QB * RC
    NB = (R - TP) // TB
    assert TP + NB * TB == R and B == 2 and TP < T
    gq = (T - TP) // RC
    bnd_it, bnd_q = gq // QB, gq % QB
    HR = max(TP, TB) + 16
    X1 = TP + 8 * NB
    XN = TB - 8

    def kernel(x_hbm, w1_hbm, dw_hbm, w2_hbm, o_hbm,
               xbuf, w1raw, w2raw, dwraw, w1p, dwb, h_ref, obuf,
               wsa, wsm, xs_all, xr_all, ss_all, g_all, wsa2, x2_all, t_all, sem_in, sem_x, sem_out):
        j = pl.program_id(0)
        sub8 = jax.lax.broadcasted_iota(jnp.int32, (8, 128), 0)
        never = sub8 > j + 1000
        xs_ref, xr_ref, ss_ref, g_ref = xs_all.at[j % 2], xr_all.at[j % 2], ss_all.at[j % 2], g_all.at[j % 2]

        def pin(v, dep):
            if dep is None:
                return v
            if v.shape[0] == 8:
                return jnp.where(never, dep, v)
            return jnp.concatenate([jnp.where(never, dep, v[0:8]), v[8:]], axis=0)

        def st_packed(ref, r, t, v):
            ref[r:r + 8, t * 128:(t + 1) * 128] = pltpu.bitcast(v.astype(bf16), u32)

        def w1_copy(col, s):
            return pltpu.make_async_copy(w1_hbm.at[:, pl.ds(col * 128, 128)], w1raw.at[col], sem_in.at[s])

        def w2_copy(col, s):
            return pltpu.make_async_copy(w2_hbm.at[:, pl.ds(col * 128, 128)], w2raw.at[col], sem_in.at[s])

        def x_copy(lo, hi, s):
            return pltpu.make_async_copy(x_hbm.at[pl.ds(lo, hi - lo), :], xbuf.at[pl.ds(lo, hi - lo), :], sem_in.at[s])

        groups = [
            [x_copy(0, XA, 0), w1_copy(0, 0), w1_copy(NC, 0)],
            [x_copy(XA, X0, 1), pltpu.make_async_copy(dw_hbm, dwraw, sem_in.at[1])],
            [w1_copy(1, 2), w1_copy(NC + 1, 2)],
            [w1_copy(2, 3), w1_copy(NC + 2, 3), w1_copy(3, 3), w1_copy(NC + 3, 3)],
            [x_copy(X0, X1, 4)] + [w2_copy(n, 4) for n in range(NC)],
        ]

        def xb_copy(i):
            lo = X1 + i * XN
            if not isinstance(lo, int):
                lo = pl.multiple_of(lo, 8)
            return pltpu.make_async_copy(x_hbm.at[pl.ds(lo, XN), :], xbuf.at[pl.ds(lo, XN), :], sem_x)

        class ctx:
            xv, ov, obase, masks, direct, xrr = xbuf, obuf, 0, {}, (), 2 * RING

        def start_group(g):
            for cp in groups[g]:
                cp.start()

        def wait_group(g):
            for cp in groups[g]:
                cp.wait()

        def w1tile(col, raw=False):
            if raw:
                wt = w1raw[col]
                if col == 0 or col >= NC:
                    w1p[:, col * 128:(col + 1) * 128] = pltpu.bitcast(wt, u32)
                return wt
            return pltpu.bitcast(w1p[:, col * 128:(col + 1) * 128], bf16)

        sub16 = jax.lax.broadcasted_iota(jnp.int32, (16, 128), 0)

        def conv16(c, o, dep, ws):
            mode, flag = ctx.masks.get(o, (None, None))
            acc = None
            for k in range(K):
                v = h_ref[c, pl.ds(8 + o + k - pad, 16), :]
                if mode == 'last' and k > pad:
                    v = jnp.where(sub16 < jnp.where(flag, 16 + pad - k, 16), v, 0.0)
                elif mode == 'first' and k < pad:
                    v = jnp.where(sub16 >= jnp.where(flag, pad - k, 0), v, 0.0)
                w = jnp.concatenate([pin(ws[k], dep) if k == K - 1 else ws[k]] * 2, axis=0)
                t = v * w
                acc = t if acc is None else acc + t
            return acc + acc * jnp.tanh(acc)

        sv = {}

        def cpair(p, l, i, half, deps):
            for u in range(2):
                c16(p, l, i, half, u, deps[u])

        def c16(p, l, i, half, u, dep):
            c = T12[half][l]
            y = conv16(c, (2 * p + u) * RC + 16 * i, dep, [dwb[c * K + k] for k in range(K)])

            def put(n, v):
                st_packed(ss_ref, ((p % RING) * 7 + n) * RH + 8 * i, l, v)
            s = sv.setdefault((p, l, i), {})
            s[(u, half)] = y
            if (u, half) == (0, 0):
                put(2, y)
            elif (u, half) == (1, 0):
                put(5, y - s[(0, 0)])
            elif (u, half) == (0, 1):
                put(4, s[(0, 0)] + y)
            else:
                put(0, s[(0, 0)] + y)
                put(1, s[(1, 0)] + y)
                put(3, y)
                put(6, s[(0, 1)] - y)
                del sv[(p, l, i)]

        def xprep(p, i, l, dep):
            def ld(q, t):
                r = q * RC + 8 + 16 * i
                cs = slice(t * 128, (t + 1) * 128)
                return jnp.concatenate([ctx.xv[r:r + 8, cs].astype(f32), ctx.xv[r + 8:r + 16, cs].astype(f32)], axis=0)
            q1, q2 = 2 * p, 2 * p + 1
            a11, a12, a21, a22 = pin(ld(q1, l), dep), ld(q1, l + 2), ld(q2, l), pin(ld(q2, l + 2), dep)
            for n, v in enumerate([a11 + a22, a21 + a22, a11 + a12, a21 - a11, a12 - a22]):
                st_packed(xs_ref, ((p % RING) * 5 + n) * RH + 8 * i, l, v)
            for u, t, v in [(0, l, a11), (0, l + 2, a12), (1, l, a21), (1, l + 2, a22)]:
                st_packed(xr_ref, ((p % RING) * 2 + u) * RH + 8 * i, t, v)

        def wprep(which, l, kl, i, dep):
            if which == 'a':
                raw, dst, kt, nt = w1raw, wsa, ((0, 1), (2, 3)), T12
            else:
                raw, dst, kt, nt = w2raw, wsm, T12, ((0, 2), (1, 3))

            def ld(kh, nh):
                r = kt[kh][kl] * 128 + 16 * i
                return raw[nt[nh][l], r:r + 16, :].astype(f32)
            b11, b12, b21, b22 = pin(ld(0, 0), dep), ld(0, 1), ld(1, 0), pin(ld(1, 1), dep)
            for n, v in enumerate([b11 + b22, b11, b12 - b22, b21 - b11, b22, b11 + b12, b21 + b22]):
                st_packed(dst, n * 128 + kl * 64 + 8 * i, l, v)

        def whalf(c, i, dep):
            for r in range(64 * i, 64 * i + 64, 16):
                st_packed(w1p, r // 2, c, pin(w1raw[NC + c, r:r + 16, :].astype(f32), dep) * 0.5)

        def comb(coef, vals):
            pos_ = [v for s, v in zip(coef, vals) if s > 0]
            neg_ = [v for s, v in zip(coef, vals) if s < 0]
            acc = pos_[0]
            for v in pos_[1:]:
                acc = acc + v
            for v in neg_:
                acc = acc - v
            return acc

        def leaves(S, X, deps, emit):
            if deps is not None:
                for k, (o, n) in enumerate(((3, 3), (3, 0), (0, 3), (0, 0))):
                    X[o][n] = pin(X[o][n], deps[k])
            for I in (3, 1, 6, 2, 0, 4, 5):
                O = [comb(S[I], [X[o][n] for o in range(4)]) for n in range(4)]
                for J in (3, 1, 6, 2, 0, 4, 5):
                    emit(I, J, comb(S[J], O))

        x2_ref, t_ref = x2_all.at[j % 2], t_all.at[j % 2]

        def xmega(Q, i, deps):
            def ld(o, n):
                q = 4 * Q + 2 * (o // 2) + n // 2
                t = 2 * (o % 2) + n % 2
                r = q * RC + 8 + 16 * i
                cs = slice(t * 128, (t + 1) * 128)
                return jnp.concatenate([ctx.xv[r:r + 8, cs].astype(f32), ctx.xv[r + 8:r + 16, cs].astype(f32)], axis=0)
            X = [[ld(o, n) for n in range(4)] for o in range(4)]

            def emit(I, J, v):
                if not (I in (2, 3) and J in (2, 3)):
                    st_packed(x2_ref, ((Q % QRING) * 25 + (7 * I + J) // 2) * RH + 8 * i, (7 * I + J) % 2, v)
            leaves(SA, X, deps, emit)

        def xraw(Q):
            for q in range(4 * Q, 4 * Q + 4):
                r = (q % XRR) * RH
                xr_ref[r:r + RH, :] = pltpu.bitcast(ctx.xv[q * RC + 8:(q + 1) * RC + 8, :], u32)

        def wmega(i, deps):
            def ld(o, n):
                r = (2 * (o // 2) + n // 2) * 128 + 16 * i
                return w1raw[2 * (o % 2) + n % 2, r:r + 16, :].astype(f32)
            X = [[ld(o, n) for n in range(4)] for o in range(4)]
            leaves(SB, X, deps, lambda I, J, v: st_packed(wsa2, (7 * I + J) // 2 * 64 + 8 * i, (7 * I + J) % 2, v))

        slot = [0]
        inner, outer = {}, {}

        def keep(name, v):
            slot[0] = (slot[0] + 1) % 40
            t_ref[slot[0] * RC:(slot[0] + 1) * RC, :] = v
            outer[name] = slot[0]

        def get(name):
            s = outer[name]
            return t_ref[s * RC:(s + 1) * RC, :]

        def fin2(Q, o, n, v):
            q = 4 * Q + 2 * (o // 2) + n // 2
            c = 2 * (o % 2) + n % 2
            g = g_ref[(q % 4) * RC:(q % 4 + 1) * RC, c * 128:(c + 1) * 128]
            h_ref[c, 16 + q * RC:16 + (q + 1) * RC, :] = v * g

        def outer_step(Q, I, n, m):
            if I == 1:
                keep(('m2', n), m)
            elif I == 3:
                fin2(Q, 2, n, get(('m2', n)) + m)
                keep(('t11', n), m)
            elif I == 2:
                keep(('m3', n), m)
                keep(('t22', n), m - get(('m2', n)))
            elif I == 4:
                fin2(Q, 1, n, get(('m3', n)) + m)
                keep(('t11', n), get(('t11', n)) - m)
            elif I == 0:
                keep(('t11', n), get(('t11', n)) + m)
                keep(('t22', n), get(('t22', n)) + m)
            elif I == 6:
                fin2(Q, 0, n, get(('t11', n)) + m)
            else:
                fin2(Q, 3, n, get(('t22', n)) + m)

        def leaf_job(Q, I, J):
            e = 7 * I + J
            if I in (2, 3) and J in (2, 3):
                o, n = 3 * (I - 2), 3 * (J - 2)
                q = 4 * Q + 2 * (o // 2) + n // 2
                t = 2 * (o % 2) + n % 2
                r = (q % XRR) * RH
                a = xr_ref[r:r + RH, t * 128:(t + 1) * 128]
            else:
                r = ((Q % QRING) * 25 + e // 2) * RH
                a = x2_ref[r:r + RH, (e % 2) * 128:(e % 2 + 1) * 128]
            w = wsa2[e // 2 * 64:(e // 2 + 1) * 64, (e % 2) * 128:(e % 2 + 1) * 128]
            m = jnp.dot(pltpu.bitcast(a, bf16), pltpu.bitcast(w, bf16), preferred_element_type=f32)
            s = inner
            if J == 1:
                s['m2'] = m
            elif J == 3:
                outer_step(Q, I, 2, s['m2'] + m)
                s['t11'] = m
            elif J == 2:
                s['m3'] = m
                s['t22'] = m - s.pop('m2')
            elif J == 4:
                outer_step(Q, I, 1, s.pop('m3') + m)
                s['t11'] = s['t11'] - m
            elif J == 0:
                s['t11'] = s['t11'] + m
                s['t22'] = s['t22'] + m
            elif J == 6:
                outer_step(Q, I, 0, s.pop('t11') + m)
            else:
                outer_step(Q, I, 3, s.pop('t22') + m)
            return m

        def lhs(kind, p, n):
            pr = p % RING
            if kind == 'm':
                v = ss_ref[(pr * 7 + n) * RH:(pr * 7 + n + 1) * RH, :]
            elif n == 2:
                v = xr_ref[2 * pr * RH:(2 * pr + 1) * RH, 0:256]
            elif n == 3:
                v = xr_ref[(2 * pr + 1) * RH:(2 * pr + 2) * RH, 256:512]
            else:
                m = {0: 0, 1: 1, 4: 2, 5: 3, 6: 4}[n]
                v = xs_ref[(pr * 5 + m) * RH:(pr * 5 + m + 1) * RH, :]
            return pltpu.bitcast(v, bf16)

        def prod(kind, p, n, l):
            w = wsa if kind == 'a' else wsm
            wt = w[n * 128:(n + 1) * 128, :] if l is None else w[n * 128:(n + 1) * 128, l * 128:(l + 1) * 128]
            return jnp.dot(lhs(kind, p, n), pltpu.bitcast(wt, bf16), preferred_element_type=f32)

        def fin(kind, p, l, rh, ch, v):
            q = 2 * p + rh
            if kind == 'a':
                c = T12[ch][l]
                g = g_ref[(q % 4) * RC:(q % 4 + 1) * RC, c * 128:(c + 1) * 128]
                h_ref[c, 16 + q * RC:16 + (q + 1) * RC, :] = v * g
            else:
                c = 2 * l + ch
                ctx.ov[q * RC:(q + 1) * RC, c * 128:(c + 1) * 128] = v.astype(bf16)

        st = {}

        bres = {}

        def run(kind, p, idx):
            if kind == 'b' and ctx.xrr == XRR and p not in ctx.direct:
                k = 8 * (p % 2) + idx
                if k % 4 == 0:
                    r, c = (2 * (p - p % 2) % XRR) * RH, k // 4
                    xq = pltpu.bitcast(xr_ref[r:r + 4 * RH, :], bf16)
                    b = jnp.dot(xq, w1tile(c), preferred_element_type=f32)
                    g_ref[:, c * 128:(c + 1) * 128] = 1.0 + jnp.tanh(b)
                    bres[0] = b
                return bres[0][(k % 4) * RC:(k % 4 + 1) * RC]
            if kind == 'b':
                u, c = idx % 2, BORD[idx]
                q = 2 * p + u
                if p in ctx.direct:
                    xq = ctx.xv[q * RC + 8:(q + 1) * RC + 8, :]
                else:
                    r = (q % ctx.xrr) * RH
                    xq = pltpu.bitcast(xr_ref[r:r + RH, :], bf16)
                b = jnp.dot(xq, w1tile(NC + c), preferred_element_type=f32)
                g_ref[(q % 4) * RC:(q % 4 + 1) * RC, c * 128:(c + 1) * 128] = 1.0 + jnp.tanh(0.5 * b)
                return b
            l = 0 if idx < 3 else 1
            step = idx if idx < 3 else idx - 4
            if idx == 3:
                m6 = prod(kind, p, 5, None)
                fin(kind, p, 0, 1, 1, st.pop('t22') + m6[:, 0:128])
                st['t22'] = m6[:, 128:256]
                return m6[:, 128:256]
            if step == 0:
                m2, m4 = prod(kind, p, 1, l), prod(kind, p, 3, l)
                fin(kind, p, l, 1, 0, m2 + m4)
                st['t11'] = m4
                st['t22'] = m2 if l == 0 else st['t22'] - m2
                return m4
            if step == 1:
                m3, m5 = prod(kind, p, 2, l), prod(kind, p, 4, l)
                fin(kind, p, l, 0, 1, m3 + m5)
                st['t11'] = st['t11'] - m5
                st['t22'] = m3 - st['t22'] if l == 0 else st['t22'] + m3
                return m5
            m1, m7 = prod(kind, p, 0, l), prod(kind, p, 6, l)
            fin(kind, p, l, 0, 0, st.pop('t11') + m1 + m7)
            if l == 0:
                st['t22'] = st['t22'] + m1
            else:
                fin(kind, p, l, 1, 1, st.pop('t22') + m1)
            return m7

        def out_dma(p, cols):
            dst = ctx.obase + 2 * p * RC
            if not isinstance(dst, int):
                dst = pl.multiple_of(dst, 16)
            pltpu.make_async_copy(ctx.ov.at[pl.ds(2 * p * RC, 2 * RC), cols],
                                  o_hbm.at[pl.ds(dst, 2 * RC), cols], sem_out).start()

        def anchors(res, n):
            nv = res.shape[0] // 8
            ks = [((2 * k + 1) * nv) // (2 * n) for k in range(n)]
            return [res[8 * k:8 * k + 8] for k in ks]

        def pipeline(groups_, p0, ns, todo):
            seq = [(kind, p, i) for kind, p in groups_ for i in range(8 if kind == 'b' else 7)]
            pos = {it: t for t, it in enumerate(seq)}
            sm, cs = [], []
            for w, dl in (('a', pos[('a', p0, 0)]), ('m', pos[('m', 0, 0)])):
                sm += [(0, dl - XDL, wprep, (w, l, kl, i)) for l in range(2) for kl in range(2) for i in range(8)]
            for p in range(p0, ns):
                dl = pos[('a' if p in ctx.direct else 'b', p, 0)] - XDL
                av = pos[('a', p - RING, 6)] + 1 if p - RING >= p0 else 0
                sm += [(av, dl, xprep, (p, i, l)) for i in range(NPAIR) for l in range(2)]
            sm += [(0, len(seq) - 10, whalf, (c, i)) for c in range(NC) for i in range(8)]
            sm.sort(key=lambda it: it[1])
            cs += [(0, pos[('m', it[0], 0)] - SDL, it) for it in todo]
            for p in range(p0, ns):
                for l in range(2):
                    for i in IORD:
                        for half in range(2):
                            av = pos[('a', p, (2 + half) if l == 0 else 6)] + SLAG
                            cs.append((av, pos[('m', p, 0)] - SDL, (p, l, i, half)))

            def plan(rate):
                out, kc, ks, credit, worst = [], 0, 0, 0.0, 0
                for t in range(len(seq)):
                    c_slack = min([it[1] - t - i for i, it in enumerate(cs[kc:kc + 80])], default=99)
                    s_slack = min([it[1] - t - i // XU for i, it in enumerate(sm[ks:ks + 80])], default=99)
                    nc = len([it for it in cs[kc:kc + (2 if c_slack < 0 else 1)] if it[0] <= t])
                    if s_slack <= 0 and c_slack > 0:
                        nc = 0
                    if nc == 0 or s_slack <= 0:
                        nx = XU0 if (t < 15 and nc == 0) else XU
                    else:
                        credit = min(credit + rate, 1.5)
                        nx = 1 if credit >= 1.0 else 0
                    nx = len([it for it in sm[ks:ks + nx] if it[0] <= t])
                    if nc:
                        credit -= min(nx, 1)
                    worst += (nc > 1) + (nc > 0 and nx > 1)
                    out.append((nc, nx))
                    kc += nc
                    ks += nx
                    assert (kc == len(cs) or cs[kc][1] > t) and (ks == len(sm) or sm[ks][1] > t)
                return worst, out
            plans = [plan(r / 100.0) for r in range(0, 101, 2)]
            best = min(w for w, o in plans)
            sched = next(o for w, o in plans if w == best)

            for t, (kind, p, idx) in enumerate(seq):
                res = run(kind, p, idx)
                nc, nx = sched[t]
                if len(seq) - 9 <= t < len(seq) - 1:
                    wmega(t - (len(seq) - 9), anchors(res, 4))
                if nc + nx:
                    an = anchors(res, 2 * nc + nx)
                    for k in range(nx):
                        it = sm.pop(0)
                        it[2](*it[3], an[k])
                    for k in range(nc):
                        cpair(*cs.pop(0)[2], an[nx + 2 * k:nx + 2 * k + 2])
            assert not sm and not cs
            n = 2 * ns * RC
            for c in range(NC):
                h_ref[c, 0:16, :] = h_ref[c, n:n + 16, :]

        def pipeline2(nq):
            jobs = [(Q, I, J) for Q in range(nq) for I in MORD for J in MORD]
            ap = [jobs[k:k + 4] for k in range(0, len(jobs), 4)]
            ns = 2 * nq
            seq, mdone = [], 0
            for Q in range(nq):
                seq += [('b', 2 * Q + k // 8, k % 8) for k in range(16)]
                seq += [('A', k, 0) for k in range(len(ap)) if ap[k][0][0] == Q]
                for p in (2 * (Q - LAGQ), 2 * (Q - LAGQ) + 1):
                    if p >= 0 and 7 * (ns - 1 - p) > RESV:
                        seq += [('m', p, i) for i in range(7)]
                        mdone = p + 1
            seq += [('m', p, i) for p in range(mdone, ns) for i in range(7)]
            pos = {it: t for t, it in enumerate(seq)}
            jpos = {jb: pos[('A', k, 0)] for k, js in enumerate(ap) for jb in js}
            lastp = {2: 3, 1: 4, 0: 6, 3: 5}
            tfin = {}
            for Q in range(nq):
                for o in range(4):
                    for n in range(4):
                        tfin[(4 * Q + 2 * (o // 2) + n // 2, 2 * (o % 2) + n % 2)] = jpos[(Q, lastp[o], lastp[n])]
            quads = []
            for p in range(ns):
                for l in range(2):
                    for i in IORD:
                        qs = [2 * p, 2 * p + 1] + ([2 * p - 1] if i == 0 and p > 0 else [])
                        av = max(tfin[(q, 2 * l + h)] for q in qs for h in range(2)) + SLAG
                        quads.append((av, pos[('m', p, 0)] - SDL, p, l, i))
            quads.sort(key=lambda it: it[0])
            cs = [(av, dl, (p, l, i, half, u)) for av, dl, p, l, i in quads for half in range(2) for u in range(2)]
            xat = {}
            free = [t for t in range(16) if t % 4 != 3]
            for Q in range(nq):
                for i in range(NPAIR):
                    if free and Q < QRING:
                        t = free.pop(0)
                    else:
                        t = pos[('b', 2 * (Q - 1), 0)] + XPOS[i]
                    assert t <= jpos[(Q, MORD[0], MORD[0])] - XDL and t not in xat
                    assert Q < QRING or t > jpos[(Q - QRING, MORD[6], MORD[6])]
                    xat[t] = (Q, i)

            icost = (20, 0, 10, 10, 20, 10, 10)
            ocost = (20, 0, 10, 20, 30, 20, 20)
            own = []
            for t, (kind, p, idx) in enumerate(seq):
                if kind == 'b':
                    v = 50
                elif kind == 'm':
                    v = (40, 60, 60, 40, 50, 60, 70)[idx]
                else:
                    v = sum(icost[J] + (ocost[I] if J in (3, 4, 5, 6) else 0) for _, I, J in ap[p])
                own.append(v + (191 if t in xat else 0))

            def plan(rate):
                out, kc, credit = [], 0, 0.0
                for t in range(len(seq)):
                    credit = min(credit, 35.0) + rate - own[t]
                    n = max(0, min(3, int(credit / 69.0 + 0.5)))
                    n = next((k for k, it in enumerate(cs[kc:kc + n]) if it[0] > t), min(n, len(cs) - kc))
                    credit -= 69.0 * n
                    out.append(n)
                    kc += n
                    if any(it[1] <= t for it in cs[kc:kc + 200]):
                        return None
                return out
            rate, sched = next((r, o) for r, o in ((r, plan(r)) for r in range(180, 320)) if o is not None)

            for t, (kind, p, idx) in enumerate(seq):
                if kind == 'b' and idx == 0 and p % 2 == 0:
                    if p == 0:
                        xraw(0)
                    if p // 2 + 1 < nq:
                        xraw(p // 2 + 1)
                if kind == 'A':
                    for k_ in list(inner):
                        if isinstance(inner[k_], tuple):
                            inner[k_] = get(inner[k_])
                    res = [leaf_job(*jb) for jb in ap[p]][-1]
                    for k_ in range(4 - len(ap[p])):
                        fill = jnp.dot(pltpu.bitcast(xr_ref[0:RH, 128 * k_:128 * k_ + 128], bf16),
                                       pltpu.bitcast(wsm[0:64, 0:128], bf16), preferred_element_type=f32)
                        keep(('fill', k_), fill)
                        res = fill
                    if seq[t + 1][0] != 'A':
                        for k_ in list(inner):
                            keep(('in', k_), inner[k_])
                            inner[k_] = ('in', k_)
                else:
                    res = run(kind, p, idx)
                if t in xat:
                    xmega(*xat[t], anchors(res, 4))
                n = sched[t]
                if n:
                    an = anchors(res, n)
                    for k in range(n):
                        c16(*cs.pop(0)[2], an[k])
                if kind == 'm':
                    if p == ns - 1:
                        if idx == 3:
                            out_dma(p, pl.ds(0, 256))
                        elif idx == 6:
                            out_dma(p, pl.ds(256, 256))
                    elif idx == 6:
                        out_dma(p, slice(None))
            assert not cs
            n = 2 * ns * RC
            for c in range(NC):
                h_ref[c, 0:16, :] = h_ref[c, n:n + 16, :]

        @pl.when(j == 0)
        def _():
            for g in range(5):
                start_group(g)
            xbuf[R:R + 16, :] = jnp.zeros((16, D), bf16)
            for c in range(NC):
                h_ref[c, 0:8, :] = jnp.zeros((8, 128), f32)

            todo = []

            def attach(res, n):
                n = min(n, len(todo))
                if n:
                    an = anchors(res, 2 * n)
                    for k in range(n):
                        cpair(*todo.pop(0), an[2 * k:2 * k + 2])

            def pw1_rows(c, lo=0, hi=X0, raw=True):
                xq = xbuf[lo:hi, :]
                a = jnp.dot(xq, w1tile(c, raw), preferred_element_type=f32)
                attach(a, 3 * P0)
                b = jnp.dot(xq, w1tile(NC + c, raw), preferred_element_type=f32)
                attach(b[0:hi - lo - 80], 2 * P0)
                g = a * (1.0 + jnp.tanh(0.5 * b))
                n = min(hi, X0 - 8) - lo
                h_ref[c, 8 + lo:8 + lo + n, :] = g[0:n]
                if hi == X0:
                    todo.extend((p, c // 2, i, c % 2) for p in range(P0) for i in IORD)

            wait_group(0)
            pw1_rows(0, 0, XA)
            wait_group(1)
            pw1_rows(0, XA, X0, raw=False)
            dwf = dwraw[...].astype(f32) * 0.25
            for c in range(NC):
                for k in range(K):
                    dwb[c * K + k] = jnp.broadcast_to(dwf[k:k + 1, c * 128:(c + 1) * 128], (8, 128))
            wait_group(2)
            xb_copy(0).start()
            pw1_rows(1)
            wait_group(3)
            pw1_rows(2)
            pw1_rows(3)
            wait_group(4)

            ctx.direct = (P0, P0 + 1)
            pipeline([(s[0], int(s[1:])) for s in PSEQ.split('.')], P0, QP // 2, todo)
            pltpu.make_async_copy(obuf.at[pl.ds(0, TP), :], o_hbm.at[pl.ds(0, TP), :], sem_out).start()

        @pl.when(j > 0)
        def _():
            i = j - 1
            xb_copy(i).wait()

            @pl.when(j < NB)
            def _():
                xb_copy(j).start()

            base = pl.multiple_of(TP + i * TB, 16)
            masks = {}
            last_flag = i == NB - 1
            if bnd_q == 0:
                last_flag = jnp.logical_or(last_flag, i == bnd_it - 1)
            else:
                masks[bnd_q * RC - 16] = ('last', i == bnd_it)
            masks[TB - 16] = ('last', last_flag)
            masks[bnd_q * RC] = ('first', i == bnd_it)
            ctx.xv, ctx.ov = xbuf.at[pl.ds(base, TB + 16), :], obuf.at[pl.ds(base, TB), :]
            ctx.obase, ctx.masks, ctx.direct, ctx.xrr = base, masks, (0, 1), XRR
            pipeline2(QB // 4)

        @pl.when(j == NB)
        def _():
            pltpu.make_async_copy(o_hbm, o_hbm, sem_out).wait()

    opts = dict(dimension_semantics=("arbitrary",), vmem_limit_bytes=100 * 1024 * 1024)
    for name in ("disable_bounds_checks", "disable_semaphore_checks"):
        if hasattr(pltpu.CompilerParams, name):
            opts[name] = True

    out = pl.pallas_call(
        kernel,
        grid=(NB + 1,),
        in_specs=[pl.BlockSpec(memory_space=pl.ANY)] * 4,
        out_specs=pl.BlockSpec(memory_space=pl.ANY),
        out_shape=jax.ShapeDtypeStruct((R, D), x.dtype),
        scratch_shapes=[
            pltpu.VMEM((R + 16, D), bf16),
            pltpu.VMEM((2 * NC, D, 128), bf16),
            pltpu.VMEM((NC, D, 128), bf16),
            pltpu.VMEM((K, D), bf16),
            pltpu.VMEM((D // 2, 2 * D), u32),
            pltpu.VMEM((NC * K, 8, 128), f32),
            pltpu.VMEM((NC, HR, 128), f32),
            pltpu.VMEM((R, D), bf16),
            pltpu.VMEM((7 * 128, 256), u32),
            pltpu.VMEM((7 * 128, 256), u32),
            pltpu.VMEM((2, RING * 5 * RH, 256), u32),
            pltpu.VMEM((2, RING * 2 * RH, D), u32),
            pltpu.VMEM((2, RING * 7 * RH, 256), u32),
            pltpu.VMEM((2, 4 * RC, D), f32),
            pltpu.VMEM((25 * 64, 256), u32),
            pltpu.VMEM((2, QRING * 25 * RH, 256), u32),
            pltpu.VMEM((2, 40 * RC, 128), f32),
            pltpu.SemaphoreType.DMA((5,)),
            pltpu.SemaphoreType.DMA,
            pltpu.SemaphoreType.DMA,
        ],
        compiler_params=pltpu.CompilerParams(**opts),
    )(x.reshape(R, D), w_pw1, dw, w_pw2)
    return out.reshape(B, T, D)
```

```python
import jax
import jax.numpy as jnp
import jax.experimental.pallas as pl
import jax.experimental.pallas.tpu as pltpu

RC = 80
NP = 6
XA = 176
QP = 12
QB = 44
PSEQ = 'b3.b4.a3.a4.b5.a5.m0.m1.m2.m3.m4.m5'
LAGQ = 1
RESV = 35
SDL = 2
SLAG = 2
XDL = 2
RING = 12
QRING = 3
XRR = 8
XPOS = (1, 4, 7, 10, 13)
BORD = (0, 1, 2, 3, 1, 0, 3, 2)
IORD = (0, 2, 4, 1, 3)
T12 = ((0, 2), (1, 3))
SA = ((1, 0, 0, 1), (0, 0, 1, 1), (1, 0, 0, 0), (0, 0, 0, 1), (1, 1, 0, 0), (-1, 0, 1, 0), (0, 1, 0, -1))
SB = ((1, 0, 0, 1), (1, 0, 0, 0), (0, 1, 0, -1), (-1, 0, 1, 0), (0, 0, 0, 1), (1, 1, 0, 0), (0, 0, 1, 1))
MORD = (1, 3, 2, 4, 0, 6, 5)


@jax.jit
def pallas_standalone__conformer_conv_module__speech_kernel(x, w_pw1, dw, w_pw2):
    B, T, D = x.shape
    K = dw.shape[0]
    pad = K // 2
    R = B * T
    NC = D // 128
    P0 = NP // 2
    assert T % RC == 0 and pad <= 8 and NC == 4 and NP % 2 == 0 and QB % 4 == 0
    f32, bf16, u32 = jnp.float32, jnp.bfloat16, jnp.uint32
    NPAIR = RC // 16
    RH = RC // 2
    X0 = NP * RC + 16
    TP = QP * RC
    TB = QB * RC
    NB = (R - TP) // TB
    assert TP + NB * TB == R and B == 2 and TP < T
    gq = (T - TP) // RC
    bnd_it, bnd_q = gq // QB, gq % QB
    HR = max(TP, TB) + 16
    X1 = TP + 8 * NB
    XN = TB - 8

    def kernel(x_hbm, w1_hbm, dw_hbm, w2_hbm, o_hbm,
               xbuf, w1raw, w2raw, dwraw, w1p, dwb, h_ref, obuf,
               wsa, wsm, xs_all, xr_all, ss_all, g_all, wsa2, x2_all, t_all, dsc, sem_in, sem_x, sem_out):
        j = pl.program_id(0)
        sub8 = jax.lax.broadcasted_iota(jnp.int32, (8, 128), 0)
        never = sub8 > j + 1000
        xs_ref, xr_ref, ss_ref, g_ref = xs_all.at[j % 2], xr_all.at[j % 2], ss_all.at[j % 2], g_all.at[j % 2]

        def pin(v, dep):
            if dep is None:
                return v
            if v.shape[0] == 8:
                return jnp.where(never, dep, v)
            return jnp.concatenate([jnp.where(never, dep, v[0:8]), v[8:]], axis=0)

        def st_packed(ref, r, t, v):
            ref[r:r + 8, t * 128:(t + 1) * 128] = pltpu.bitcast(v.astype(bf16), u32)

        def w1_copy(col, s):
            return pltpu.make_async_copy(w1_hbm.at[:, pl.ds(col * 128, 128)], w1raw.at[col], sem_in.at[s])

        def w2_copy(col, s):
            return pltpu.make_async_copy(w2_hbm.at[:, pl.ds(col * 128, 128)], w2raw.at[col], sem_in.at[s])

        def x_copy(lo, hi, s):
            return pltpu.make_async_copy(x_hbm.at[pl.ds(lo, hi - lo), :], xbuf.at[pl.ds(lo, hi - lo), :], sem_in.at[s])

        groups = [
            [x_copy(0, XA, 0), w1_copy(0, 0), w1_copy(NC, 0)],
            [x_copy(XA, X0, 1), pltpu.make_async_copy(dw_hbm, dwraw, sem_in.at[1])],
            [w1_copy(1, 2), w1_copy(NC + 1, 2)],
            [w1_copy(2, 3), w1_copy(NC + 2, 3), w1_copy(3, 3), w1_copy(NC + 3, 3)],
            [x_copy(X0, X1, 4)] + [w2_copy(n, 4) for n in range(NC)],
        ]

        def xb_copy(i):
            lo = X1 + i * XN
            if not isinstance(lo, int):
                lo = pl.multiple_of(lo, 8)
            return pltpu.make_async_copy(x_hbm.at[pl.ds(lo, XN), :], xbuf.at[pl.ds(lo, XN), :], sem_x)

        class ctx:
            xv, ov, obase, masks, direct, xrr = xbuf, obuf, 0, {}, (), 2 * RING

        def start_group(g):
            for cp in groups[g]:
                cp.start()

        def wait_group(g):
            for cp in groups[g]:
                cp.wait()

        def w1tile(col, raw=False):
            if raw:
                wt = w1raw[col]
                if col == 0 or col >= NC:
                    w1p[:, col * 128:(col + 1) * 128] = pltpu.bitcast(wt, u32)
                return wt
            return pltpu.bitcast(w1p[:, col * 128:(col + 1) * 128], bf16)

        sub16 = jax.lax.broadcasted_iota(jnp.int32, (16, 128), 0)

        def conv16(c, o, dep, ws):
            mode, flag = ctx.masks.get(o, (None, None))
            acc = None
            for k in range(K):
                v = h_ref[c, pl.ds(8 + o + k - pad, 16), :]
                if mode == 'last' and k > pad:
                    v = jnp.where(sub16 < jnp.where(flag, 16 + pad - k, 16), v, 0.0)
                elif mode == 'first' and k < pad:
                    v = jnp.where(sub16 >= jnp.where(flag, pad - k, 0), v, 0.0)
                w = jnp.concatenate([pin(ws[k], dep) if k == K - 1 else ws[k]] * 2, axis=0)
                t = v * w
                acc = t if acc is None else acc + t
            return acc + acc * jnp.tanh(acc)

        sv = {}

        def cpair(p, l, i, half, deps):
            for u in range(2):
                c16(p, l, i, half, u, deps[u])

        def c16(p, l, i, half, u, dep):
            c = T12[half][l]
            y = conv16(c, (2 * p + u) * RC + 16 * i, dep, [dwb[c * K + k] for k in range(K)])

            def put(n, v):
                st_packed(ss_ref, ((p % RING) * 7 + n) * RH + 8 * i, l, v)
            s = sv.setdefault((p, l, i), {})
            s[(u, half)] = y
            if (u, half) == (0, 0):
                put(2, y)
            elif (u, half) == (1, 0):
                put(5, y - s[(0, 0)])
            elif (u, half) == (0, 1):
                put(4, s[(0, 0)] + y)
            else:
                put(0, s[(0, 0)] + y)
                put(1, s[(1, 0)] + y)
                put(3, y)
                put(6, s[(0, 1)] - y)
                del sv[(p, l, i)]

        def xprep(p, i, l, dep):
            def ld(q, t):
                r = q * RC + 8 + 16 * i
                cs = slice(t * 128, (t + 1) * 128)
                return jnp.concatenate([ctx.xv[r:r + 8, cs].astype(f32), ctx.xv[r + 8:r + 16, cs].astype(f32)], axis=0)
            q1, q2 = 2 * p, 2 * p + 1
            a11, a12, a21, a22 = pin(ld(q1, l), dep), ld(q1, l + 2), ld(q2, l), pin(ld(q2, l + 2), dep)
            for n, v in enumerate([a11 + a22, a21 + a22, a11 + a12, a21 - a11, a12 - a22]):
                st_packed(xs_ref, ((p % RING) * 5 + n) * RH + 8 * i, l, v)
            for u, t, v in [(0, l, a11), (0, l + 2, a12), (1, l, a21), (1, l + 2, a22)]:
                st_packed(xr_ref, ((p % RING) * 2 + u) * RH + 8 * i, t, v)

        def wprep(which, l, kl, i, dep):
            if which == 'a':
                raw, dst, kt, nt = w1raw, wsa, ((0, 1), (2, 3)), T12
            else:
                raw, dst, kt, nt = w2raw, wsm, T12, ((0, 2), (1, 3))

            def ld(kh, nh):
                r = kt[kh][kl] * 128 + 16 * i
                v = raw[nt[nh][l], r:r + 16, :].astype(f32)
                return v * jnp.concatenate([dsc[NC + nt[nh][l]]] * 2, axis=0) if which == 'a' else v
            b11, b12, b21, b22 = pin(ld(0, 0), dep), ld(0, 1), ld(1, 0), pin(ld(1, 1), dep)
            for n, v in enumerate([b11 + b22, b11, b12 - b22, b21 - b11, b22, b11 + b12, b21 + b22]):
                st_packed(dst, n * 128 + kl * 64 + 8 * i, l, v)

        def whalf(c, i, dep):
            for r in range(64 * i, 64 * i + 64, 16):
                st_packed(w1p, r // 2, c, pin(w1raw[NC + c, r:r + 16, :].astype(f32), dep) * 0.5)

        def comb(coef, vals):
            pos_ = [v for s, v in zip(coef, vals) if s > 0]
            neg_ = [v for s, v in zip(coef, vals) if s < 0]
            acc = pos_[0]
            for v in pos_[1:]:
                acc = acc + v
            for v in neg_:
                acc = acc - v
            return acc

        def leaves(S, X, deps, emit):
            if deps is not None:
                for k, (o, n) in enumerate(((3, 3), (3, 0), (0, 3), (0, 0))):
                    X[o][n] = pin(X[o][n], deps[k])
            for I in (3, 1, 6, 2, 0, 4, 5):
                O = [comb(S[I], [X[o][n] for o in range(4)]) for n in range(4)]
                for J in (3, 1, 6, 2, 0, 4, 5):
                    emit(I, J, comb(S[J], O))

        x2_ref, t_ref = x2_all.at[j % 2], t_all.at[j % 2]

        def xmega(Q, i, deps):
            def ld(o, n):
                q = 4 * Q + 2 * (o // 2) + n // 2
                t = 2 * (o % 2) + n % 2
                r = q * RC + 8 + 16 * i
                cs = slice(t * 128, (t + 1) * 128)
                return jnp.concatenate([ctx.xv[r:r + 8, cs].astype(f32), ctx.xv[r + 8:r + 16, cs].astype(f32)], axis=0)
            X = [[ld(o, n) for n in range(4)] for o in range(4)]

            def emit(I, J, v):
                if not (I in (2, 3) and J in (2, 3)):
                    st_packed(x2_ref, ((Q % QRING) * 25 + (7 * I + J) // 2) * RH + 8 * i, (7 * I + J) % 2, v)
            leaves(SA, X, deps, emit)

        def xraw(Q):
            for q in range(4 * Q, 4 * Q + 4):
                r = (q % XRR) * RH
                xr_ref[r:r + RH, :] = pltpu.bitcast(ctx.xv[q * RC + 8:(q + 1) * RC + 8, :], u32)

        def wmega(i, deps):
            def ld(o, n):
                r = (2 * (o // 2) + n // 2) * 128 + 16 * i
                c = 2 * (o % 2) + n % 2
                return w1raw[c, r:r + 16, :].astype(f32) * jnp.concatenate([dsc[NC + c]] * 2, axis=0)
            X = [[ld(o, n) for n in range(4)] for o in range(4)]
            leaves(SB, X, deps, lambda I, J, v: st_packed(wsa2, (7 * I + J) // 2 * 64 + 8 * i, (7 * I + J) % 2, v))

        slot = [0]
        inner, outer = {}, {}

        def keep(name, v):
            slot[0] = (slot[0] + 1) % 40
            t_ref[slot[0] * RC:(slot[0] + 1) * RC, :] = v
            outer[name] = slot[0]

        def get(name):
            s = outer[name]
            return t_ref[s * RC:(s + 1) * RC, :]

        def fin2(Q, o, n, v):
            q = 4 * Q + 2 * (o // 2) + n // 2
            c = 2 * (o % 2) + n % 2
            g = g_ref[(q % 4) * RC:(q % 4 + 1) * RC, c * 128:(c + 1) * 128]
            h_ref[c, 16 + q * RC:16 + (q + 1) * RC, :] = v * g

        def outer_step(Q, I, n, m):
            if I == 1:
                keep(('m2', n), m)
            elif I == 3:
                fin2(Q, 2, n, get(('m2', n)) + m)
                keep(('t11', n), m)
            elif I == 2:
                keep(('m3', n), m)
                keep(('t22', n), m - get(('m2', n)))
            elif I == 4:
                fin2(Q, 1, n, get(('m3', n)) + m)
                keep(('t11', n), get(('t11', n)) - m)
            elif I == 0:
                keep(('t11', n), get(('t11', n)) + m)
                keep(('t22', n), get(('t22', n)) + m)
            elif I == 6:
                fin2(Q, 0, n, get(('t11', n)) + m)
            else:
                fin2(Q, 3, n, get(('t22', n)) + m)

        def leaf_job(Q, I, J):
            e = 7 * I + J
            if I in (2, 3) and J in (2, 3):
                o, n = 3 * (I - 2), 3 * (J - 2)
                q = 4 * Q + 2 * (o // 2) + n // 2
                t = 2 * (o % 2) + n % 2
                r = (q % XRR) * RH
                a = xr_ref[r:r + RH, t * 128:(t + 1) * 128]
            else:
                r = ((Q % QRING) * 25 + e // 2) * RH
                a = x2_ref[r:r + RH, (e % 2) * 128:(e % 2 + 1) * 128]
            w = wsa2[e // 2 * 64:(e // 2 + 1) * 64, (e % 2) * 128:(e % 2 + 1) * 128]
            m = jnp.dot(pltpu.bitcast(a, bf16), pltpu.bitcast(w, bf16), preferred_element_type=f32)
            s = inner
            if J == 1:
                s['m2'] = m
            elif J == 3:
                outer_step(Q, I, 2, s['m2'] + m)
                s['t11'] = m
            elif J == 2:
                s['m3'] = m
                s['t22'] = m - s.pop('m2')
            elif J == 4:
                outer_step(Q, I, 1, s.pop('m3') + m)
                s['t11'] = s['t11'] - m
            elif J == 0:
                s['t11'] = s['t11'] + m
                s['t22'] = s['t22'] + m
            elif J == 6:
                outer_step(Q, I, 0, s.pop('t11') + m)
            else:
                outer_step(Q, I, 3, s.pop('t22') + m)
            return m

        def lhs(kind, p, n):
            pr = p % RING
            if kind == 'm':
                v = ss_ref[(pr * 7 + n) * RH:(pr * 7 + n + 1) * RH, :]
            elif n == 2:
                v = xr_ref[2 * pr * RH:(2 * pr + 1) * RH, 0:256]
            elif n == 3:
                v = xr_ref[(2 * pr + 1) * RH:(2 * pr + 2) * RH, 256:512]
            else:
                m = {0: 0, 1: 1, 4: 2, 5: 3, 6: 4}[n]
                v = xs_ref[(pr * 5 + m) * RH:(pr * 5 + m + 1) * RH, :]
            return pltpu.bitcast(v, bf16)

        def prod(kind, p, n, l):
            w = wsa if kind == 'a' else wsm
            wt = w[n * 128:(n + 1) * 128, :] if l is None else w[n * 128:(n + 1) * 128, l * 128:(l + 1) * 128]
            return jnp.dot(lhs(kind, p, n), pltpu.bitcast(wt, bf16), preferred_element_type=f32)

        def fin(kind, p, l, rh, ch, v):
            q = 2 * p + rh
            if kind == 'a':
                c = T12[ch][l]
                g = g_ref[(q % 4) * RC:(q % 4 + 1) * RC, c * 128:(c + 1) * 128]
                h_ref[c, 16 + q * RC:16 + (q + 1) * RC, :] = v * g
            else:
                c = 2 * l + ch
                ctx.ov[q * RC:(q + 1) * RC, c * 128:(c + 1) * 128] = v.astype(bf16)

        st = {}

        bres = {}

        def run(kind, p, idx):
            if kind == 'b' and ctx.xrr == XRR and p not in ctx.direct:
                k = 8 * (p % 2) + idx
                if k % 4 == 0:
                    r, c = (2 * (p - p % 2) % XRR) * RH, k // 4
                    xq = pltpu.bitcast(xr_ref[r:r + 4 * RH, :], bf16)
                    b = jnp.dot(xq, w1tile(c), preferred_element_type=f32)
                    g_ref[:, c * 128:(c + 1) * 128] = 1.0 + jnp.tanh(b)
                    bres[0] = b
                return bres[0][(k % 4) * RC:(k % 4 + 1) * RC]
            if kind == 'b':
                u, c = idx % 2, BORD[idx]
                q = 2 * p + u
                if p in ctx.direct:
                    xq = ctx.xv[q * RC + 8:(q + 1) * RC + 8, :]
                else:
                    r = (q % ctx.xrr) * RH
                    xq = pltpu.bitcast(xr_ref[r:r + RH, :], bf16)
                b = jnp.dot(xq, w1tile(NC + c), preferred_element_type=f32)
                g_ref[(q % 4) * RC:(q % 4 + 1) * RC, c * 128:(c + 1) * 128] = 1.0 + jnp.tanh(0.5 * b)
                return b
            l = 0 if idx < 3 else 1
            step = idx if idx < 3 else idx - 4
            if idx == 3:
                m6 = prod(kind, p, 5, None)
                fin(kind, p, 0, 1, 1, st.pop('t22') + m6[:, 0:128])
                st['t22'] = m6[:, 128:256]
                return m6[:, 128:256]
            if step == 0:
                m2, m4 = prod(kind, p, 1, l), prod(kind, p, 3, l)
                fin(kind, p, l, 1, 0, m2 + m4)
                st['t11'] = m4
                st['t22'] = m2 if l == 0 else st['t22'] - m2
                return m4
            if step == 1:
                m3, m5 = prod(kind, p, 2, l), prod(kind, p, 4, l)
                fin(kind, p, l, 0, 1, m3 + m5)
                st['t11'] = st['t11'] - m5
                st['t22'] = m3 - st['t22'] if l == 0 else st['t22'] + m3
                return m5
            m1, m7 = prod(kind, p, 0, l), prod(kind, p, 6, l)
            fin(kind, p, l, 0, 0, st.pop('t11') + m1 + m7)
            if l == 0:
                st['t22'] = st['t22'] + m1
            else:
                fin(kind, p, l, 1, 1, st.pop('t22') + m1)
            return m7

        def out_dma(p, cols):
            dst = ctx.obase + 2 * p * RC
            if not isinstance(dst, int):
                dst = pl.multiple_of(dst, 16)
            pltpu.make_async_copy(ctx.ov.at[pl.ds(2 * p * RC, 2 * RC), cols],
                                  o_hbm.at[pl.ds(dst, 2 * RC), cols], sem_out).start()

        def anchors(res, n):
            nv = res.shape[0] // 8
            ks = [((2 * k + 1) * nv) // (2 * n) for k in range(n)]
            return [res[8 * k:8 * k + 8] for k in ks]

        def pipeline(groups_, p0, ns, todo):
            seq = [(kind, p, i) for kind, p in groups_ for i in range(8 if kind == 'b' else 7)]
            pos = {it: t for t, it in enumerate(seq)}
            pcs = []
            for w, dl, cost in (('a', pos[('a', p0, 0)], 35), ('m', pos[('m', 0, 0)], 27)):
                pcs += [(0, dl - XDL, cost, 1, wprep, (w, l, kl, i))
                        for l in range(2) for kl in range(2) for i in range(8)]
            for p in range(p0, ns):
                dl = pos[('a' if p in ctx.direct else 'b', p, 0)] - XDL
                pcs += [(0, dl, 29, 1, xprep, (p, i, l)) for i in range(NPAIR) for l in range(2)]
            pcs += [(0, pos[('m', it[0], 0)] - SDL, 69, 1, c16, it + (u,)) for it in todo for u in range(2)]
            for p in range(p0, ns):
                for l in range(2):
                    for i in IORD:
                        for half in range(2):
                            av = pos[('a', p, (2 + half) if l == 0 else 6)] + SLAG
                            pcs += [(av, pos[('m', p, 0)] - SDL, 69, 1, c16, (p, l, i, half, u)) for u in range(2)]
            pcs += [(0, len(seq) - 2, 24, 1, whalf, (c, i)) for c in range(NC) for i in range(8)]
            pcs += [(0, len(seq) - 2, 227, 4, wmega, (i,)) for i in range(8)]
            pcs.sort(key=lambda it: it[1])
            own = [(80 if p in ctx.direct else 60) if kind == 'b' else (40, 60, 60, 40, 50, 60, 70)[idx]
                   for kind, p, idx in seq]

            def plan(rate):
                out, credit, pend = [], 0.0, list(pcs)
                for t in range(len(seq)):
                    credit = min(credit, 35.0) + rate - own[t]
                    take, blocked = [], False
                    for it in pend:
                        if it[0] > t or (blocked and it[4] is c16):
                            blocked = blocked or it[4] is c16
                            continue
                        if it[2] * (0.5 if it[2] < 100 else 0.7) > credit or len(take) == 7:
                            break
                        take.append(it)
                        credit -= it[2]
                    pend = [it for it in pend if it not in take]
                    out.append(take)
                    if pend and pend[0][1] <= t:
                        return None
                return out
            sched = next(o for o in (plan(r) for r in range(200, 400, 2)) if o is not None)

            for t, (kind, p, idx) in enumerate(seq):
                res = run(kind, p, idx)
                if sched[t]:
                    an = anchors(res, sum(it[3] for it in sched[t]))
                    for it in sched[t]:
                        it[4](*it[5], an[0] if it[3] == 1 else an[:it[3]])
                        an = an[it[3]:]
            n = 2 * ns * RC
            for c in range(NC):
                h_ref[c, 0:16, :] = h_ref[c, n:n + 16, :]

        def pipeline2(nq):
            jobs = [(Q, I, J) for Q in range(nq) for I in MORD for J in MORD]
            ap = [jobs[k:k + 4] for k in range(0, len(jobs), 4)]
            ns = 2 * nq
            seq, mdone = [], 0
            for Q in range(nq):
                seq += [('b', 2 * Q + k // 8, k % 8) for k in range(16)]
                seq += [('A', k, 0) for k in range(len(ap)) if ap[k][0][0] == Q]
                for p in (2 * (Q - LAGQ), 2 * (Q - LAGQ) + 1):
                    if p >= 0 and 7 * (ns - 1 - p) > RESV:
                        seq += [('m', p, i) for i in range(7)]
                        mdone = p + 1
            seq += [('m', p, i) for p in range(mdone, ns) for i in range(7)]
            pos = {it: t for t, it in enumerate(seq)}
            jpos = {jb: pos[('A', k, 0)] for k, js in enumerate(ap) for jb in js}
            lastp = {2: 3, 1: 4, 0: 6, 3: 5}
            tfin = {}
            for Q in range(nq):
                for o in range(4):
                    for n in range(4):
                        tfin[(4 * Q + 2 * (o // 2) + n // 2, 2 * (o % 2) + n % 2)] = jpos[(Q, lastp[o], lastp[n])]
            quads = []
            for p in range(ns):
                for l in range(2):
                    for i in IORD:
                        qs = [2 * p, 2 * p + 1] + ([2 * p - 1] if i == 0 and p > 0 else [])
                        av = max(tfin[(q, 2 * l + h)] for q in qs for h in range(2)) + SLAG
                        quads.append((av, pos[('m', p, 0)] - SDL, p, l, i))
            quads.sort(key=lambda it: it[0])
            cs = [(av, dl, (p, l, i, half, u)) for av, dl, p, l, i in quads for half in range(2) for u in range(2)]
            xat = {}
            free = [t for t in range(16) if t % 4 != 3]
            for Q in range(nq):
                for i in range(NPAIR):
                    if free and Q < QRING:
                        t = free.pop(0)
                    else:
                        t = pos[('b', 2 * (Q - 1), 0)] + XPOS[i]
                    assert t <= jpos[(Q, MORD[0], MORD[0])] - XDL and t not in xat
                    assert Q < QRING or t > jpos[(Q - QRING, MORD[6], MORD[6])]
                    xat[t] = (Q, i)

            icost = (20, 0, 10, 10, 20, 10, 10)
            ocost = (20, 0, 10, 20, 30, 20, 20)
            own = []
            for t, (kind, p, idx) in enumerate(seq):
                if kind == 'b':
                    v = 50
                elif kind == 'm':
                    v = (40, 60, 60, 40, 50, 60, 70)[idx]
                else:
                    v = sum(icost[J] + (ocost[I] if J in (3, 4, 5, 6) else 0) for _, I, J in ap[p])
                own.append(v + (191 if t in xat else 0))

            def plan(rate):
                out, kc, credit = [], 0, 0.0
                for t in range(len(seq)):
                    credit = min(credit, 35.0) + rate - own[t]
                    n = max(0, min(3, int(credit / 69.0 + 0.5)))
                    n = next((k for k, it in enumerate(cs[kc:kc + n]) if it[0] > t), min(n, len(cs) - kc))
                    credit -= 69.0 * n
                    out.append(n)
                    kc += n
                    if any(it[1] <= t for it in cs[kc:kc + 200]):
                        return None
                return out
            rate, sched = next((r, o) for r, o in ((r, plan(r)) for r in range(180, 320)) if o is not None)

            for t, (kind, p, idx) in enumerate(seq):
                if kind == 'b' and idx == 0 and p % 2 == 0:
                    if p == 0:
                        xraw(0)
                    if p // 2 + 1 < nq:
                        xraw(p // 2 + 1)
                if kind == 'A':
                    for k_ in list(inner):
                        if isinstance(inner[k_], tuple):
                            inner[k_] = get(inner[k_])
                    res = [leaf_job(*jb) for jb in ap[p]][-1]
                    for k_ in range(4 - len(ap[p])):
                        fill = jnp.dot(pltpu.bitcast(xr_ref[0:RH, 128 * k_:128 * k_ + 128], bf16),
                                       pltpu.bitcast(wsm[0:64, 0:128], bf16), preferred_element_type=f32)
                        keep(('fill', k_), fill)
                        res = fill
                    if seq[t + 1][0] != 'A':
                        for k_ in list(inner):
                            keep(('in', k_), inner[k_])
                            inner[k_] = ('in', k_)
                else:
                    res = run(kind, p, idx)
                if t in xat:
                    xmega(*xat[t], anchors(res, 4))
                n = sched[t]
                if n:
                    an = anchors(res, n)
                    for k in range(n):
                        c16(*cs.pop(0)[2], an[k])
                if kind == 'm':
                    if p == ns - 1:
                        if idx == 3:
                            out_dma(p, pl.ds(0, 256))
                        elif idx == 6:
                            out_dma(p, pl.ds(256, 256))
                    elif idx == 6:
                        out_dma(p, slice(None))
            assert not cs
            n = 2 * ns * RC
            for c in range(NC):
                h_ref[c, 0:16, :] = h_ref[c, n:n + 16, :]

        @pl.when(j == 0)
        def _():
            for g in range(5):
                start_group(g)
            xbuf[R:R + 16, :] = jnp.zeros((16, D), bf16)
            for c in range(NC):
                h_ref[c, 0:8, :] = jnp.zeros((8, 128), f32)

            todo = []

            def attach(res, n):
                n = min(n, len(todo))
                if n:
                    an = anchors(res, 2 * n)
                    for k in range(n):
                        cpair(*todo.pop(0), an[2 * k:2 * k + 2])

            def pw1_rows(c, lo=0, hi=X0, raw=True):
                xq = xbuf[lo:hi, :]
                wa = w1tile(c, raw)
                if raw:
                    acc = [None] * 2
                    for r in range(0, D, 16):
                        wf = w1raw[c, r:r + 16, :].astype(f32)
                        k = (r // 16) % 2
                        acc[k] = wf * wf if acc[k] is None else acc[k] + wf * wf
                    ss = jnp.broadcast_to(jnp.sum(acc[0] + acc[1], axis=0, keepdims=True), (8, 128))
                    if c == 0:
                        dsc[2 * NC] = jnp.broadcast_to(256.0 / jnp.sum(ss, axis=1, keepdims=True), (8, 128))
                    e = ((pltpu.bitcast(ss * dsc[2 * NC], jnp.int32) >> 23) - 127) >> 1
                    e = jnp.clip(e, -40, 40)
                    dsc[c] = pltpu.bitcast((127 + e) << 23, f32)
                    dsc[NC + c] = pltpu.bitcast((127 - e) << 23, f32)
                a = jnp.dot(xq, wa, preferred_element_type=f32)
                attach(a, 3 * P0)
                b = jnp.dot(xq, w1tile(NC + c, raw), preferred_element_type=f32)
                attach(b[0:hi - lo - 80], 2 * P0)
                dv = jnp.concatenate([dsc[NC + c]] * ((hi - lo) // 8), axis=0)
                g = a * (dv + dv * jnp.tanh(0.5 * b))
                n = min(hi, X0 - 8) - lo
                h_ref[c, 8 + lo:8 + lo + n, :] = g[0:n]
                if hi == X0:
                    dwf = dwraw[:, c * 128:(c + 1) * 128].astype(f32) * 0.25
                    for k in range(K):
                        dwb[c * K + k] = jnp.broadcast_to(dwf[k:k + 1, :], (8, 128)) * dsc[c]
                    todo.extend((p, c // 2, i, c % 2) for p in range(P0) for i in IORD)

            wait_group(0)
            pw1_rows(0, 0, XA)
            wait_group(1)
            pw1_rows(0, XA, X0, raw=False)
            wait_group(2)
            xb_copy(0).start()
            pw1_rows(1)
            wait_group(3)
            pw1_rows(2)
            pw1_rows(3)
            wait_group(4)

            ctx.direct = (P0, P0 + 1)
            pipeline([(s[0], int(s[1:])) for s in PSEQ.split('.')], P0, QP // 2, todo)
            pltpu.make_async_copy(obuf.at[pl.ds(0, TP), :], o_hbm.at[pl.ds(0, TP), :], sem_out).start()

        @pl.when(j > 0)
        def _():
            i = j - 1
            xb_copy(i).wait()

            @pl.when(j < NB)
            def _():
                xb_copy(j).start()

            base = pl.multiple_of(TP + i * TB, 16)
            masks = {}
            last_flag = i == NB - 1
            if bnd_q == 0:
                last_flag = jnp.logical_or(last_flag, i == bnd_it - 1)
            else:
                masks[bnd_q * RC - 16] = ('last', i == bnd_it)
            masks[TB - 16] = ('last', last_flag)
            masks[bnd_q * RC] = ('first', i == bnd_it)
            ctx.xv, ctx.ov = xbuf.at[pl.ds(base, TB + 16), :], obuf.at[pl.ds(base, TB), :]
            ctx.obase, ctx.masks, ctx.direct, ctx.xrr = base, masks, (0, 1), XRR
            pipeline2(QB // 4)

        @pl.when(j == NB)
        def _():
            pltpu.make_async_copy(o_hbm, o_hbm, sem_out).wait()

    opts = dict(dimension_semantics=("arbitrary",), vmem_limit_bytes=100 * 1024 * 1024)
    for name in ("disable_bounds_checks", "disable_semaphore_checks"):
        if hasattr(pltpu.CompilerParams, name):
            opts[name] = True

    out = pl.pallas_call(
        kernel,
        grid=(NB + 1,),
        in_specs=[pl.BlockSpec(memory_space=pl.ANY)] * 4,
        out_specs=pl.BlockSpec(memory_space=pl.ANY),
        out_shape=jax.ShapeDtypeStruct((R, D), x.dtype),
        scratch_shapes=[
            pltpu.VMEM((R + 16, D), bf16),
            pltpu.VMEM((2 * NC, D, 128), bf16),
            pltpu.VMEM((NC, D, 128), bf16),
            pltpu.VMEM((K, D), bf16),
            pltpu.VMEM((D // 2, 2 * D), u32),
            pltpu.VMEM((NC * K, 8, 128), f32),
            pltpu.VMEM((NC, HR, 128), f32),
            pltpu.VMEM((R, D), bf16),
            pltpu.VMEM((7 * 128, 256), u32),
            pltpu.VMEM((7 * 128, 256), u32),
            pltpu.VMEM((2, RING * 5 * RH, 256), u32),
            pltpu.VMEM((2, RING * 2 * RH, D), u32),
            pltpu.VMEM((2, RING * 7 * RH, 256), u32),
            pltpu.VMEM((2, 4 * RC, D), f32),
            pltpu.VMEM((25 * 64, 256), u32),
            pltpu.VMEM((2, QRING * 25 * RH, 256), u32),
            pltpu.VMEM((2, 40 * RC, 128), f32),
            pltpu.VMEM((2 * NC + 1, 8, 128), f32),
            pltpu.SemaphoreType.DMA((5,)),
            pltpu.SemaphoreType.DMA,
            pltpu.SemaphoreType.DMA,
        ],
        compiler_params=pltpu.CompilerParams(**opts),
    )(x.reshape(R, D), w_pw1, dw, w_pw2)
    return out.reshape(B, T, D)
```

```python
import jax
import jax.numpy as jnp
import jax.experimental.pallas as pl
import jax.experimental.pallas.tpu as pltpu

RC = 80
QP = 12
NP = 6
XA = 176
QB = 44
MLAG = 6
DEADLINE = 3


@jax.jit
def pallas_standalone__conformer_conv_module__speech_kernel(x, w_pw1, dw, w_pw2):
    B, T, D = x.shape
    K = dw.shape[0]
    pad = K // 2
    R = B * T
    NC = D // 128
    TP = QP * RC
    TB = QB * RC
    NB = (R - TP) // TB
    assert TP + NB * TB == R and T % RC == 0 and B == 2 and TP < T and pad <= 8 and NC == 4
    gq = (T - TP) // RC
    bnd_it, bnd_q = gq // QB, gq % QB
    f32, bf16, u32 = jnp.float32, jnp.bfloat16, jnp.uint32
    HR = max(TP, TB) + 16
    NPAIR = RC // 16
    X0 = NP * RC + 16
    X1 = TP + 8 * NB
    XN = TB - 8

    def kernel(x_hbm, w1_hbm, dw_hbm, w2_hbm, o_hbm,
               xbuf, w1raw, w2raw, dwraw, w1p, w2p, dwb, h_ref, s_all, obuf, sem_in, sem_x, sem_out):
        j = pl.program_id(0)
        sub = jax.lax.broadcasted_iota(jnp.int32, (16, 128), 0)
        never = sub > j + 1000
        s_ref = s_all.at[j % 2]

        def w1_copy(col, s):
            return pltpu.make_async_copy(w1_hbm.at[:, pl.ds(col * 128, 128)], w1raw.at[col], sem_in.at[s])

        def w2_copy(col, s):
            return pltpu.make_async_copy(w2_hbm.at[:, pl.ds(col * 128, 128)], w2raw.at[col], sem_in.at[s])

        def x_copy(lo, hi, s):
            return pltpu.make_async_copy(x_hbm.at[pl.ds(lo, hi - lo), :], xbuf.at[pl.ds(lo, hi - lo), :], sem_in.at[s])

        groups = [
            [x_copy(0, XA, 0), w1_copy(0, 0), w1_copy(NC, 0)],
            [x_copy(XA, X0, 1), pltpu.make_async_copy(dw_hbm, dwraw, sem_in.at[1])],
            [w1_copy(1, 2), w1_copy(NC + 1, 2)],
            [w1_copy(2, 3), w1_copy(NC + 2, 3), w1_copy(3, 3), w1_copy(NC + 3, 3)],
            [w2_copy(n, 4) for n in range(NC)] + [x_copy(X0, X1, 4)],
        ]

        def wait_group(g):
            for cp in groups[g]:
                cp.wait()

        def xb_copy(i):
            lo = X1 + i * XN
            if not isinstance(lo, int):
                lo = pl.multiple_of(lo, 8)
            return pltpu.make_async_copy(x_hbm.at[pl.ds(lo, XN), :], xbuf.at[pl.ds(lo, XN), :], sem_x)

        def w1tile(col, raw=False):
            if raw:
                wt = w1raw[col]
                w1p[:, col * 128:(col + 1) * 128] = pltpu.bitcast(wt, u32)
                return wt
            return pltpu.bitcast(w1p[:, col * 128:(col + 1) * 128], bf16)

        def w2tile(col, raw=False):
            if raw:
                wt = w2raw[col]
                w2p[:, col * 128:(col + 1) * 128] = pltpu.bitcast(wt, u32)
                return wt
            return pltpu.bitcast(w2p[:, col * 128:(col + 1) * 128], bf16)

        def conv16(c, o, mode, flag, dep, kdep, ws):
            acc = None
            for k in range(K):
                v = h_ref[c, pl.ds(8 + o + k - pad, 16), :]
                if mode == 'last' and k > pad:
                    v = jnp.where(sub < jnp.where(flag, 16 + pad - k, 16), v, 0.0)
                elif mode == 'first' and k < pad:
                    v = jnp.where(sub >= jnp.where(flag, pad - k, 0), v, 0.0)
                w = ws[k]
                if k == kdep and dep is not None:
                    w = jnp.where(never, dep, w)
                t = v * w
                acc = t if acc is None else acc + t
            return acc + acc * jnp.tanh(acc)

        class Blk:
            def __init__(self, xv, ov, obase, masks, kdep):
                self.xv, self.ov, self.obase, self.masks, self.kdep = xv, ov, obase, masks, kdep
                self.raw_w2 = False
                self.nq = 0
                self.xq, self.r, self.av, self.ws = {}, {}, {}, {}
                self.todo = []

            def conv_pair(self, q, c, p, dep):
                o = q * RC + 16 * p
                mode, flag = self.masks.get((q, p), (None, None))
                if (q, c) not in self.ws:
                    self.ws[(q, c)] = [jnp.concatenate([dwb[c * K + k]] * 2, axis=0) for k in range(K)]
                sp = conv16(c, o, mode, flag, dep, self.kdep, self.ws[(q, c)]).astype(bf16)
                s_ref[o // 2:o // 2 + 8, c * 128:(c + 1) * 128] = pltpu.bitcast(sp, u32)

            def attach(self, res, npairs):
                nv = res.shape[0] // 8
                npairs = min(npairs, len(self.todo))
                for i in range(npairs):
                    q, c, p = self.todo.pop(0)
                    i0 = (2 * i * nv) // (2 * npairs)
                    i1 = ((2 * i + 1) * nv) // (2 * npairs)
                    dep = jnp.concatenate([res[8 * i0:8 * i0 + 8], res[8 * i1:8 * i1 + 8]], axis=0)
                    self.conv_pair(q, c, p, dep)

            def run(self, kind, q, c, npairs):
                if kind == 'a':
                    if q not in self.xq:
                        self.xq[q] = self.xv[q * RC + 8:(q + 1) * RC + 8, :]
                    a = jnp.dot(self.xq[q], w1tile(c), preferred_element_type=f32)
                    self.av[(q, c)] = a
                    self.attach(a, npairs)
                elif kind == 'b':
                    b = jnp.dot(self.xq[q], w1tile(NC + c), preferred_element_type=f32)
                    self.attach(b, npairs)
                    h_ref[c, 16 + q * RC:16 + (q + 1) * RC, :] = self.av.pop((q, c)) * (1.0 + jnp.tanh(0.5 * b))
                    self.todo.extend((q, c, p) for p in range(NPAIR))
                else:
                    n = c
                    while any(it[0] <= q for it in self.todo):
                        self.conv_pair(*self.todo.pop(0), None)
                    s = pltpu.bitcast(s_ref[q * RC // 2:(q + 1) * RC // 2, :], bf16)
                    r = jnp.dot(s, w2tile(n, self.raw_w2 and q == 0), preferred_element_type=f32)
                    self.attach(r, npairs)
                    if n % 2 == 0:
                        self.r[q] = r
                    else:
                        self.ov[q * RC:(q + 1) * RC, (n - 1) * 128:(n + 1) * 128] = (
                            jnp.concatenate([self.r.pop(q), r], axis=1).astype(bf16))
                    if not isinstance(self.obase, int):
                        dst = pl.multiple_of(self.obase + q * RC, 16)
                        if q == self.nq - 1:
                            if n % 2 == 1:
                                cols = pl.ds((n - 1) * 128, 256)
                                pltpu.make_async_copy(self.ov.at[pl.ds(q * RC, RC), cols],
                                                      o_hbm.at[pl.ds(dst, RC), cols], sem_out).start()
                        elif n == NC - 1:
                            pltpu.make_async_copy(self.ov.at[pl.ds(q * RC, RC), :],
                                                  o_hbm.at[pl.ds(dst, RC), :], sem_out).start()

            def steady(self, q0, nq, pending):
                self.nq = nq
                seq = []
                ready = {q: MLAG - 1 for q in pending}
                pend = [(q, n) for q in pending for n in range(NC)]
                for q in range(q0, nq):
                    for c in range(NC):
                        seq.append(('a', q, c))
                        seq.append(('b', q, c))
                        if c == NC - 1:
                            ready[q] = len(seq) - 1 + MLAG
                            pend += [(q, n) for n in range(NC)]
                        k = 2 if len(pend) > 2 * NC + 2 else 1
                        if q == nq - 1:
                            k = 0 if len(pend) <= NC + (NC if c == NC - 1 else 0) else k
                        for _ in range(k):
                            if pend and ready[pend[0][0]] <= len(seq):
                                seq.append(('m',) + pend.pop(0))
                for it in pend:
                    seq.append(('m',) + it)
                first_m = {}
                for t, (kind, q, c) in enumerate(seq):
                    if kind == 'm' and q not in first_m:
                        first_m[q] = t
                for t, (kind, q, c) in enumerate(seq):
                    base = 1 if kind == 'b' else 2
                    n = base
                    if self.todo:
                        need = 0
                        for idx, it in enumerate(self.todo):
                            slots = max(first_m[it[0]] - DEADLINE - t + 1, 1)
                            need = max(need, -(-(idx + 1) // slots))
                        n = max(base, min(base + 2, need))
                        if len(self.todo) > 8:
                            n = max(n, base + 1)
                    self.run(kind, q, c, n)

            def carry(self, n):
                for c in range(NC):
                    h_ref[c, 0:16, :] = h_ref[c, n:n + 16, :]

        @pl.when(j == 0)
        def _():
            for g in groups:
                for cp in g:
                    cp.start()
            xbuf[R:R + 16, :] = jnp.zeros((16, D), bf16)
            for c in range(NC):
                h_ref[c, 0:8, :] = jnp.zeros((8, 128), f32)
            blk = Blk(xbuf, obuf, 0, {}, K - 1)

            def pw1_rows(c, lo=0, hi=X0, raw=True):
                xq = xbuf[lo:hi, :]
                a = jnp.dot(xq, w1tile(c, raw), preferred_element_type=f32)
                blk.attach(a, 3 * NP)
                b = jnp.dot(xq, w1tile(NC + c, raw), preferred_element_type=f32)
                blk.attach(b[0:hi - lo - 80], 2 * NP)
                g = a * (1.0 + jnp.tanh(0.5 * b))
                n = min(hi, X0 - 8) - lo
                h_ref[c, 8 + lo:8 + lo + n, :] = g[0:n]
                if hi == X0:
                    blk.todo.extend((q, c, p) for q in range(NP) for p in range(NPAIR))

            wait_group(0)
            pw1_rows(0, 0, XA)
            wait_group(1)
            pw1_rows(0, XA, X0, raw=False)
            dwf = dwraw[...].astype(f32) * 0.25
            for c in range(NC):
                for k in range(K):
                    dwb[c * K + k] = jnp.broadcast_to(dwf[k:k + 1, c * 128:(c + 1) * 128], (8, 128))
            wait_group(2)
            pw1_rows(1)
            wait_group(3)
            xb_copy(0).start()
            pw1_rows(2)
            pw1_rows(3)
            wait_group(4)
            blk.raw_w2 = True
            blk.steady(NP, QP, list(range(NP)))
            blk.carry(TP)
            pltpu.make_async_copy(obuf.at[pl.ds(0, TP), :], o_hbm.at[pl.ds(0, TP), :], sem_out).start()

        @pl.when(j > 0)
        def _():
            i = j - 1
            xb_copy(i).wait()

            @pl.when(j < NB)
            def _():
                xb_copy(j).start()

            base = pl.multiple_of(TP + i * TB, 16)
            masks = {}
            last_flag = i == NB - 1
            if bnd_q == 0:
                last_flag = jnp.logical_or(last_flag, i == bnd_it - 1)
            else:
                masks[(bnd_q - 1, NPAIR - 1)] = ('last', i == bnd_it)
            masks[(QB - 1, NPAIR - 1)] = ('last', last_flag)
            masks[(bnd_q, 0)] = ('first', i == bnd_it)
            b = Blk(xbuf.at[pl.ds(base, TB + 16), :], obuf.at[pl.ds(base, TB), :], base, masks, 0)
            b.steady(0, QB, [])
            b.carry(TB)

        @pl.when(j == NB)
        def _():
            pltpu.make_async_copy(o_hbm, o_hbm, sem_out).wait()

    opts = dict(dimension_semantics=("arbitrary",), vmem_limit_bytes=100 * 1024 * 1024)
    for name in ("disable_bounds_checks", "disable_semaphore_checks"):
        if hasattr(pltpu.CompilerParams, name):
            opts[name] = True

    out = pl.pallas_call(
        kernel,
        grid=(NB + 1,),
        in_specs=[pl.BlockSpec(memory_space=pl.ANY)] * 4,
        out_specs=pl.BlockSpec(memory_space=pl.ANY),
        out_shape=jax.ShapeDtypeStruct((R, D), x.dtype),
        scratch_shapes=[
            pltpu.VMEM((R + 16, D), bf16),
            pltpu.VMEM((2 * NC, D, 128), bf16),
            pltpu.VMEM((NC, D, 128), bf16),
            pltpu.VMEM((K, D), bf16),
            pltpu.VMEM((D // 2, 2 * D), u32),
            pltpu.VMEM((D // 2, D), u32),
            pltpu.VMEM((NC * K, 8, 128), f32),
            pltpu.VMEM((NC, HR, 128), f32),
            pltpu.VMEM((2, max(TP, TB) // 2, D), u32),
            pltpu.VMEM((R, D), bf16),
            pltpu.SemaphoreType.DMA((5,)),
            pltpu.SemaphoreType.DMA,
            pltpu.SemaphoreType.DMA,
        ],
        compiler_params=pltpu.CompilerParams(**opts),
    )(x.reshape(R, D), w_pw1, dw, w_pw2)
    return out.reshape(B, T, D)
```
